```python
import os as _os
_os.environ.setdefault("JAX_PLATFORMS", "cpu")
import jax
import jax.numpy as jnp

def _softmax(x, axis=-1):
    return jax.nn.softmax(x, axis=axis)
def _gelu(x):
    return jax.nn.gelu(x, approximate=True)
def _silu(x):
    return jax.nn.silu(x)
def _sigmoid(x):
    return jax.nn.sigmoid(x)
def _layernorm(x, axis=-1, eps=1e-5):
    m = jnp.mean(x, axis=axis, keepdims=True)
    v = jnp.var(x, axis=axis, keepdims=True)
    return (x - m) / jnp.sqrt(v + eps)
def _scatter_add(tgt, idx, src, axis=0):
    return tgt.at[idx].add(src)
def _segment_sum(src, seg, n):
    return jax.ops.segment_sum(src, seg, n)
class _Rng:
    def __init__(self, key):
        self._k = key
    def _next(self):
        self._k, sub = jax.random.split(self._k)
        return sub
    def normal(self, shape):
        return jax.random.normal(self._next(), shape, dtype=jnp.bfloat16)
    def randint(self, lo, hi, shape):
        return jax.random.randint(self._next(), shape, lo, hi, dtype=jnp.int32)
    def uniform(self, shape, lo=0.0, hi=1.0):
        return jax.random.uniform(self._next(), shape, jnp.bfloat16, lo, hi)
    def permutation(self, n):
        return jax.random.permutation(self._next(), n)


kernel_name = 'gated_mix__linear_attn_block__mixer_token_mlp__prompt'

def setup_inputs():
    _rng = _Rng(jax.random.key(int.from_bytes(__import__("os").urandom(4), "little")))
    _w = (lambda a: (lambda t: t.astype(jnp.bfloat16) if jnp.issubdtype(t.dtype, jnp.floating) else t)(jnp.asarray(a)))
    def _A_setup():
        B, S, D = 1, 2048, 512
        return {
            "x": _w((lambda *s: _rng.normal(s) * 0.05)(B, S, D)),
            "wqkv": _w((lambda *s: _rng.normal(s) * 0.8)(D, 3 * D)),
            "wo": _w((lambda *s: _rng.normal(s) * 0.05)(D, D)),
        }
    _A_in = _A_setup()

    def _B_setup():
        B, S, D, F = 1, 2048, 512, 1792
        return {
            "x": _w((lambda *s: _rng.normal(s) * 0.05)(B, S, D)),
            "w1": _w((lambda *s: _rng.normal(s) * 0.1)(S, F) * (S ** -0.5)),
            "b1": _w((lambda *s: _rng.normal(s) * 0.1)(F) * 0.02),
            "w2": _w((lambda *s: _rng.normal(s) * 0.1)(F, S) * (F ** -0.5)),
            "b2": _w((lambda *s: _rng.normal(s) * 0.1)(S) * 0.02),
        }
    _B_in = _B_setup()

    return {
        "A_x": _A_in["x"],
        "A_wqkv": _A_in["wqkv"],
        "A_wo": _A_in["wo"],
        "B_x": _B_in["x"],
        "B_w1": _B_in["w1"],
        "B_b1": _B_in["b1"],
        "B_w2": _B_in["w2"],
        "B_b2": _B_in["b2"],
        "gate_w": _w((lambda *s: _rng.normal(s) * 0.05)(512) * 16.0),
    }

def reference(A_x, A_wqkv, A_wo, B_x, B_w1, B_b1, B_w2, B_b2, gate_w):
    def _A_ref(x, wqkv, wo):
        B, S, D = x.shape
        H = 32; Dh = D // H
        qkv = (lambda x, *d: x.transpose(*d))((x @ wqkv).reshape(B, S, 3, H, Dh), 2, 0, 3, 1, 4)
        q, k, v = qkv[0], qkv[1], qkv[2]
        phi = lambda t: jnp.where(t > 0, t + 1, jnp.exp(t)) + 1e-6
        pq, pk = phi(q), phi(k)
        kv = jnp.einsum("bhsd,bhse->bhde", pk, v)
        z = jnp.einsum("bhsd->bhd", pk)
        num = jnp.einsum("bhqd,bhde->bhqe", pq, kv)
        den = jnp.einsum("bhqd,bhd->bhq", pq, z)[..., None] + 1e-6
        o = num / den
        return (lambda x, *d: x.transpose(*d))(o, 0, 2, 1, 3).reshape(B, S, D) @ wo

    def _B_ref(x, w1, b1, w2, b2):
        B, S, D = x.shape
        h = _layernorm(x, axis=-1)
        u = jnp.einsum("bsd,sf->bdf", h, w1) + b1
        u = _gelu(u)
        y = jnp.einsum("bdf,fs->bds", u, w2) + b2
        return (lambda x, *d: x.transpose(*d))(y, 0, 2, 1)

    x = A_x
    g = _sigmoid((x * gate_w).sum(-1, keepdims=True))
    a = _A_ref(x, A_wqkv, A_wo)
    b = _B_ref(x, B_w1, B_b1, B_w2, B_b2)
    return g * a + (1 - g) * b
```

```python
import jax, jax.numpy as jnp, numpy as np
from jax import lax
from jax.experimental import pallas as pl
from jax.experimental.pallas import tpu as pltpu

S, D, F, H, DH = 2048, 512, 1792, 32, 16
bf16, f32 = jnp.bfloat16, jnp.float32

def phi(t):
    return jnp.where(t > 0, t + 1.0, jnp.exp(t)) + 1e-6

def gelu(u):
    c = float(np.sqrt(2.0 / np.pi))
    return 0.5 * u * (1.0 + jnp.tanh(c * (u + 0.044715 * (u * u * u))))

def dot(a, b):
    return jnp.dot(a, b, preferred_element_type=f32)

NC = 4
CS = S // NC
NB = 4
SB = S // NB

def kernel(x_hbm, wqkv_hbm, wo_hbm, w1_hbm, b1_hbm, w2_hbm, b2_hbm, gw_hbm, out_hbm,
           x_v, wqkv_v, wo_v, w1_v, w2_v, b1_v, b2_v, gw_v,
           xT_v, hT_v, pk_v, pq_v, uT_v, out_v, sems, osems):
    cp = pltpu.make_async_copy
    x_cp = [cp(x_hbm.at[pl.ds(c * CS, CS)], x_v.at[pl.ds(c * CS, CS)], sems.at[c]) for c in range(NC)]
    wk_cp = cp(wqkv_hbm.at[:, pl.ds(D, D)], wqkv_v.at[1], sems.at[NC])
    wq_cp = cp(wqkv_hbm.at[:, pl.ds(0, D)], wqkv_v.at[0], sems.at[NC + 1])
    wv_cp = cp(wqkv_hbm.at[:, pl.ds(2 * D, D)], wqkv_v.at[2], sems.at[NC + 2])
    wo_cp = cp(wo_hbm, wo_v, sems.at[NC + 3])
    w1_cp = cp(w1_hbm, w1_v, sems.at[NC + 4])
    w2_cp = cp(w2_hbm, w2_v, sems.at[NC + 5])
    b1_cp = cp(b1_hbm, b1_v, sems.at[NC + 6])
    b2_cp = cp(b2_hbm, b2_v, sems.at[NC + 7])
    gw_cp = cp(gw_hbm, gw_v, sems.at[NC + 8])

    wk_cp.start()
    x_cp[0].start()
    gw_cp.start()
    for c in range(1, NC):
        x_cp[c].start()
    wk_cp.wait()
    gw_cp.wait()
    wq_cp.start(); wv_cp.start(); wo_cp.start()
    b1_cp.start(); b2_cp.start()
    w1_cp.start(); w2_cp.start()

    gw = gw_v[...].astype(f32).reshape(1, D)
    gwT = jnp.broadcast_to(gw, (128, D)).T
    wk = wqkv_v[1]
    GT = jnp.zeros((D, D), f32)
    z = jnp.zeros((1, D), f32)
    gates = []
    for c in range(NC):
        x_cp[c].wait()
        xc = x_v[pl.ds(c * CS, CS), :]
        k = dot(xc, wk)
        pk = phi(k)
        z = z + jnp.sum(pk, axis=0, keepdims=True)
        pkb = pk.astype(bf16)
        xTc = xc.T
        xT_v[:, pl.ds(c * CS, CS)] = xTc
        GT = GT + dot(xTc, pkb)
        xf = xTc.astype(f32)
        m = jnp.mean(xf, axis=0, keepdims=True)
        xm = xf - m
        var = jnp.mean(xm * xm, axis=0, keepdims=True)
        hT_v[:, pl.ds(c * CS, CS)] = (xm / jnp.sqrt(var + 1e-5)).astype(bf16)
        gsum = jnp.sum(xf * jnp.tile(gwT, (1, CS // 128)), axis=0, keepdims=True)
        gates.append(jax.nn.sigmoid(gsum))

    wq_cp.wait(); wv_cp.wait(); wo_cp.wait()
    wqT = wqkv_v[0].T
    wvT = wqkv_v[2].T
    woT = wo_v[...].T
    GTb = GT.astype(bf16)
    zT = jnp.broadcast_to(z, (128, D)).T
    r = lax.broadcasted_iota(jnp.int32, (128, 128), 0) // DH
    cc = lax.broadcasted_iota(jnp.int32, (128, 128), 1) // DH
    msk = r == cc
    MT = []
    for b in range(D // 128):
        sl = slice(b * 128, (b + 1) * 128)
        kvT = dot(wvT[sl, :], GTb[:, sl])
        kvT = jnp.where(msk, kvT, 0.0).astype(bf16)
        MT.append(dot(woT[:, sl], kvT).astype(bf16))
    MT = jnp.concatenate(MT, axis=1)

    for c in range(NC):
        qT = dot(wqT, xT_v[:, pl.ds(c * CS, CS)])
        pq = phi(qT)
        t = pq * jnp.tile(zT, (1, CS // 128))
        den = jnp.sum(t.reshape(H, DH, CS), axis=1, keepdims=True) + 1e-6
        pqn = pq.reshape(H, DH, CS) / den
        pq_v[:, pl.ds(c * CS, CS)] = pqn.reshape(D, CS).astype(bf16)

    b1_cp.wait(); b2_cp.wait()
    w1_cp.wait()
    b1 = b1_v[...].astype(f32).reshape(1, F)
    b2 = b2_v[...].astype(f32).reshape(1, S)
    u = dot(hT_v[...], w1_v[...]) + b1
    uT_v[...] = gelu(u).astype(bf16)

    w2_cp.wait()
    o_cp = []
    for b in range(NB):
        sl = pl.ds(b * SB, SB)
        yT = dot(uT_v[...], w2_v[:, sl]) + b2[:, b * SB:(b + 1) * SB]
        aT = dot(MT, pq_v[:, sl])
        g = gates[b]
        oT = g * aT + (1.0 - g) * yT
        out_v[sl, :] = oT.astype(bf16).T
        c = cp(out_v.at[sl], out_hbm.at[sl], osems.at[b])
        c.start()
        o_cp.append(c)
    for c in o_cp:
        c.wait()

@jax.jit
def pallas_gated_mix__linear_attn_block__mixer_token_mlp__prompt_kernel(A_x, A_wqkv, A_wo, B_x, B_w1, B_b1, B_w2, B_b2, gate_w):
    x = A_x.reshape(S, D)
    anyspec = pl.BlockSpec(memory_space=pl.ANY)
    out = pl.pallas_call(
        kernel,
        out_shape=jax.ShapeDtypeStruct((S, D), bf16),
        in_specs=[anyspec] * 8,
        out_specs=anyspec,
        scratch_shapes=[
            pltpu.VMEM((S, D), bf16), pltpu.VMEM((3, D, D), bf16), pltpu.VMEM((D, D), bf16),
            pltpu.VMEM((S, F), bf16), pltpu.VMEM((F, S), bf16),
            pltpu.VMEM((F,), bf16), pltpu.VMEM((S,), bf16), pltpu.VMEM((D,), bf16),
            pltpu.VMEM((D, S), bf16), pltpu.VMEM((D, S), bf16), pltpu.VMEM((S, D), bf16),
            pltpu.VMEM((D, S), bf16), pltpu.VMEM((D, F), bf16), pltpu.VMEM((S, D), bf16),
            pltpu.SemaphoreType.DMA((NC + 9,)), pltpu.SemaphoreType.DMA((NB,)),
        ],
        compiler_params=pltpu.CompilerParams(vmem_limit_bytes=100 << 20),
    )(x, A_wqkv, A_wo, B_w1, B_b1, B_w2, B_b2, gate_w)
    return out.reshape(1, S, D)
```

```python
import jax, jax.numpy as jnp, numpy as np
from jax import lax
from jax.experimental import pallas as pl
from jax.experimental.pallas import tpu as pltpu

S, D, F, H, DH = 2048, 512, 1792, 32, 16
bf16, f32 = jnp.bfloat16, jnp.float32

def phi(t):
    return jnp.where(t > 0, t + 1.0, jnp.exp(t)) + 1e-6

def gelu(u):
    c = float(np.sqrt(2.0 / np.pi))
    return (0.5 * u) * (1.0 + jnp.tanh(u * (c + (c * 0.044715) * (u * u))))

def dot(a, b):
    return jnp.dot(a, b, preferred_element_type=f32)

def dot_nt(a, b):
    return lax.dot_general(a, b, (((1,), (1,)), ((), ())), preferred_element_type=f32)

def recip(d):
    r = pl.reciprocal(d, approx=True)
    return r * (2.0 - d * r)

CH = [(0, 256), (256, 512), (768, 1280)]
TS = 128
GK = 2
NBLK = [(i * 256, 256) for i in range(6)] + [(1536, 128), (1664, 128), (1792, 128), (1920, 128)]
LG = 32
PROG = [("wx", 0), ("k", 0), ("ln", 0), ("k", 1), ("ln", 1), ("g", 0, 2),
        ("wx", 1), ("wq",), ("k", 2), ("ln", 2), ("k", 3), ("ln", 3), ("q", 0), ("k", 4), ("ln", 4), ("q", 1), ("k", 5), ("ln", 5), ("q", 2), ("q", 3), ("g", 2, 4),
        ("wx", 2), ("wvo",)]
for j in range(6, 14, 4):
    PROG += [("k", j), ("ln", j), ("q", j - 2), ("k", j + 1), ("ln", j + 1), ("q", j - 1), ("k", j + 2), ("ln", j + 2), ("q", j), ("k", j + 3), ("ln", j + 3), ("q", j + 1), ("g", j, 4)]
PROG += [("k", 14), ("ln", 14), ("q", 12), ("k", 15), ("ln", 15), ("q", 13), ("g", 14, 2), ("q", 14), ("small",), ("small2",), ("qdot", 15), ("w3",), ("qstore", 15)]
PROG2 = []
for i in range(7):
    PROG2 += [("b1", i * 256, 256)]
    if i < 6: PROG2 += [("pqa", i * 256, 256)]
FENCES = [8]
PROG3 = {0: [(1536, 256)], 1: [(1792, 256)]}

def kernel(x_hbm, wqkv_hbm, wo_hbm, w1_hbm, b1_hbm, w2_hbm, b2_hbm, gw_hbm, out_hbm,
           x_v, wqkv_v, wo_v, w1_v, w2_v, b1_v, b2_v, gw_v,
           wkT_v, wqT_v, MT_v, hT_v, q_v, pn_v, pk_v, a_v, uT_v, out_v, sems, osems, rsem):
    cp = pltpu.make_async_copy
    NC = len(CH)
    x_cp = [cp(x_hbm.at[pl.ds(s, n)], x_v.at[pl.ds(s, n)], sems.at[c]) for c, (s, n) in enumerate(CH)]
    wk_cp = cp(wqkv_hbm.at[:, pl.ds(D, D)], wqkv_v.at[1], sems.at[NC])
    wq_cp = cp(wqkv_hbm.at[:, pl.ds(0, D)], wqkv_v.at[0], sems.at[NC + 1])
    wv_cp = cp(wqkv_hbm.at[:, pl.ds(2 * D, D)], wqkv_v.at[2], sems.at[NC + 2])
    wo_cp = cp(wo_hbm, wo_v, sems.at[NC + 3])
    w1_cp = cp(w1_hbm, w1_v, sems.at[NC + 4])
    w2_cp = cp(w2_hbm, w2_v, sems.at[NC + 5])
    b1_cp = cp(b1_hbm, b1_v, sems.at[NC + 6])
    b2_cp = cp(b2_hbm, b2_v, sems.at[NC + 7])
    gw_cp = cp(gw_hbm, gw_v, sems.at[NC + 8])

    gw_cp.start(); wk_cp.start(); x_cp[0].start(); wq_cp.start(); x_cp[1].start()
    wv_cp.start(); wo_cp.start()
    for c in range(2, NC):
        x_cp[c].start()
    b1_cp.start(); b2_cp.start()
    w1_cp.start(); w2_cp.start()
    gw_cp.wait(); wk_cp.wait()
    gw = gw_v[...].astype(f32).reshape(1, D)
    wkT_v[...] = wqkv_v[1].T

    st = dict(G=None, z=None)
    glog = []

    def k_step(t0):
        rows = pl.ds(t0, TS)
        kT = dot_nt(wkT_v[...], x_v[rows, :])
        pk = phi(kT)
        st["z"] = pk if st["z"] is None else st["z"] + pk
        pk_v[:, rows] = pk.astype(bf16)

    def ln_step(t0):
        hs, gls = [], []
        for r0 in range(0, TS, LG):
            xf = x_v[pl.ds(t0 + r0, LG), :].astype(f32)
            m = jnp.sum(xf, axis=1, keepdims=True) * (1.0 / D)
            gls.append(jnp.sum(xf * gw, axis=1, keepdims=True))
            xm = xf - m
            var = jnp.sum(xm * xm, axis=1, keepdims=True) * (1.0 / D)
            hs.append(xm * lax.rsqrt(var + 1e-5))
        h = jnp.concatenate(hs, axis=0)
        gl = jnp.concatenate(gls, axis=0)
        hT_v[:, pl.ds(t0, TS)] = h.T.astype(bf16)
        glog.append(jnp.broadcast_to(gl, (TS, 128)).T[0:1, :])

    def q_step(t0):
        rows = pl.ds(t0, TS)
        q_v[:, rows] = dot_nt(wqT_v[...], x_v[rows, :]).astype(bf16)

    def g_step(t0, n):
        gr = pl.ds(t0, n)
        gc = dot(pk_v[:, gr], x_v[gr, :])
        st["G"] = gc if st["G"] is None else st["G"] + gc

    def small_chain():
        woT = wo_v[...].T
        Gb = st["G"].astype(bf16)
        r = lax.broadcasted_iota(jnp.int32, (128, 128), 0) // DH
        cc = lax.broadcasted_iota(jnp.int32, (128, 128), 1) // DH
        msk = r == cc
        kvs = []
        for b in range(D // 128):
            sl = slice(b * 128, (b + 1) * 128)
            kv = dot(Gb[sl, :], wqkv_v[2, :, sl])
            kvs.append(jnp.where(msk, kv, 0.0).astype(bf16))
        st["kvs"] = kvs
        st["woT"] = woT

    def small_chain2():
        for b in range(D // 128):
            sl = slice(b * 128, (b + 1) * 128)
            MT_v[:, sl] = dot_nt(st["woT"][:, sl], st["kvs"][b]).astype(bf16)

    for op in PROG:
        if op[0] == "wx":
            x_cp[op[1]].wait()
        elif op[0] == "wq":
            wq_cp.wait()
            wqT_v[...] = wqkv_v[0].T
        elif op[0] == "wvo":
            wv_cp.wait(); wo_cp.wait()
        elif op[0] == "k":
            k_step(op[1] * TS)
        elif op[0] == "ln":
            ln_step(op[1] * TS)
        elif op[0] == "q":
            q_step(op[1] * TS)
        elif op[0] == "g":
            g_step(op[1] * TS, op[2] * TS)
        elif op[0] == "small":
            small_chain()
        elif op[0] == "small2":
            small_chain2()
        elif op[0] == "qdot":
            st["qv"] = dot_nt(wqT_v[...], x_v[pl.ds(op[1] * TS, TS), :])
        elif op[0] == "qstore":
            q_v[:, pl.ds(op[1] * TS, TS)] = st["qv"].astype(bf16)
        elif op[0] == "w3":
            b1_cp.wait(); b2_cp.wait(); w1_cp.wait()
    glog = [glog[i] for i in np.argsort([o[1] for o in PROG if o[0] == "ln"])]
    g_all = jax.nn.sigmoid(jnp.concatenate(glog, axis=1))
    zT = jnp.broadcast_to(jnp.sum(st["z"], axis=1, keepdims=True), (D, 128))

    b1 = b1_v[...].astype(f32).reshape(1, F)
    b2 = b2_v[...].astype(f32).reshape(1, S)

    def pqn_step(s0, cs):
        ql = pl.ds(s0, cs)
        pq = phi(q_v[:, ql].astype(f32))
        t = pq * jnp.tile(zT, (1, cs // 128))
        den = jnp.sum(t.reshape(H, DH, cs), axis=1, keepdims=True) + 1e-6
        pqn = pq.reshape(H, DH, cs) * recip(den)
        pn_v[:, ql] = pqn.reshape(D, cs).astype(bf16)

    def pqa_step(s0, cs):
        ql = pl.ds(s0, cs)
        pq = phi(q_v[:, ql].astype(f32))
        t = pq * jnp.tile(zT, (1, cs // 128))
        den = jnp.sum(t.reshape(H, DH, cs), axis=1, keepdims=True) + 1e-6
        pqn = pq.reshape(H, DH, cs) * recip(den)
        a_v[:, ql] = dot(MT_v[...], pqn.reshape(D, cs).astype(bf16)) * g_all[:, s0:s0 + cs]

    def a_step(s0, cs):
        ql = pl.ds(s0, cs)
        a_v[:, ql] = dot(MT_v[...], pn_v[:, ql]) * g_all[:, s0:s0 + cs]

    for op in PROG2:
        if op[0] == "b1":
            sl = pl.ds(op[1], op[2])
            u = dot(hT_v[...], w1_v[:, sl]) + b1[:, op[1]:op[1] + op[2]]
            if op[1] + op[2] == F:
                w2_cp.wait()
            uT_v[:, sl] = gelu(u).astype(bf16)
        elif op[0] == "pq":
            pqn_step(op[1], op[2])
        elif op[0] == "a":
            a_step(op[1], op[2])
        elif op[0] == "pqa":
            pqa_step(op[1], op[2])

    o_cp = []
    started = 0
    waited = 0
    for b, (s0, sb) in enumerate(NBLK):
        sl = pl.ds(s0, sb)
        if b in FENCES:
            for c in o_cp[started:]:
                c.start()
            started = len(o_cp)
            pl.semaphore_signal(rsem, 1)
            pl.semaphore_wait(rsem, 1)
        yT = dot(uT_v[...], w2_v[:, sl]) + b2[:, s0:s0 + sb]
        for q0, qn in PROG3.get(b, []):
            pqa_step(q0, qn)
        g = g_all[:, s0:s0 + sb]
        oT = a_v[:, sl] + (1.0 - g) * yT
        out_v[sl, :] = oT.T.astype(bf16)
        o_cp.append(cp(out_v.at[sl], out_hbm.at[sl], osems.at[b]))
    for c in o_cp[started:]:
        c.start()
    for c in o_cp:
        c.wait()

@jax.jit
def pallas_gated_mix__linear_attn_block__mixer_token_mlp__prompt_kernel(A_x, A_wqkv, A_wo, B_x, B_w1, B_b1, B_w2, B_b2, gate_w):
    x = A_x.reshape(S, D)
    anyspec = pl.BlockSpec(memory_space=pl.ANY)
    out = pl.pallas_call(
        kernel,
        out_shape=jax.ShapeDtypeStruct((S, D), bf16),
        in_specs=[anyspec] * 8,
        out_specs=anyspec,
        scratch_shapes=[
            pltpu.VMEM((S, D), bf16), pltpu.VMEM((3, D, D), bf16), pltpu.VMEM((D, D), bf16),
            pltpu.VMEM((S, F), bf16), pltpu.VMEM((F, S), bf16),
            pltpu.VMEM((F,), bf16), pltpu.VMEM((S,), bf16), pltpu.VMEM((D,), bf16),
            pltpu.VMEM((D, D), bf16), pltpu.VMEM((D, D), bf16), pltpu.VMEM((D, D), bf16),
            pltpu.VMEM((D, S), bf16), pltpu.VMEM((D, S), bf16), pltpu.VMEM((D, S), bf16), pltpu.VMEM((D, S), bf16), pltpu.VMEM((D, S), f32),
            pltpu.VMEM((D, F), bf16), pltpu.VMEM((S, D), bf16),
            pltpu.SemaphoreType.DMA((len(CH) + 9,)), pltpu.SemaphoreType.DMA((len(NBLK),)), pltpu.SemaphoreType.REGULAR(()),
        ],
        compiler_params=pltpu.CompilerParams(vmem_limit_bytes=100 << 20),
    )(x, A_wqkv, A_wo, B_w1, B_b1, B_w2, B_b2, gate_w)
    return out.reshape(1, S, D)
```

```python
import jax, jax.numpy as jnp, numpy as np
from jax import lax
from jax.experimental import pallas as pl
from jax.experimental.pallas import tpu as pltpu

S, D, F, H, DH = 2048, 512, 1792, 32, 16
HD = D // 2
bf16, f32, u32 = jnp.bfloat16, jnp.float32, jnp.uint32

def phi(t):
    return jnp.where(t > 0, t + 1.0, jnp.exp(t)) + 1e-6

def gelu(u):
    c = float(np.sqrt(2.0 / np.pi))
    return (0.5 * u) * (1.0 + jnp.tanh(u * (c + (c * 0.044715) * (u * u))))

def dot(a, b):
    return jnp.dot(a, b, preferred_element_type=f32)

def dot_nt(a, b):
    return lax.dot_general(a, b, (((1,), (1,)), ((), ())), preferred_element_type=f32)

def recip(d):
    r = pl.reciprocal(d, approx=True)
    return r * (2.0 - d * r)

def B(v):
    return pltpu.bitcast(v, bf16)

def U(v):
    return pltpu.bitcast(v.astype(bf16), u32)

def rs(s0, n):
    return pl.ds(s0 // 2, n // 2)

CH = [(0, 256), (256, 512), (768, 1280)]
TS = 128
LG = 32
PROG = [("wx", 0), ("k", 0), ("k", 1), ("g", 0, 2),
        ("wx", 1), ("wq",), ("k", 2), ("ln", 0), ("k", 3), ("ln", 1), ("k", 4), ("ln", 2), ("q", 0), ("k", 5), ("ln", 3), ("q", 1), ("q", 2), ("ln", 4), ("q", 3), ("ln", 5), ("q", 4), ("q", 5), ("g", 2, 4),
        ("wx", 2), ("wvo",)]
for j in range(6, 14, 4):
    PROG += [("k", j), ("ln", j), ("k", j + 1), ("ln", j + 1), ("q", j), ("k", j + 2), ("ln", j + 2), ("q", j + 1), ("k", j + 3), ("ln", j + 3), ("q", j + 2), ("q", j + 3), ("g", j, 4)]
PROG += [("k", 14), ("ln", 14), ("k", 15), ("ln", 15), ("q", 14), ("q", 15), ("g", 14, 2)]
W2PAIR = 4
SMALL = {0: {2: "small", 4: "small2"}}
HOOKPOS = (2, 4)
FENCES = {6: 4, 7: 4}

def kernel(x_hbm, wqkv_hbm, wo_hbm, w1_hbm, b1_hbm, w2_hbm, b2_hbm, gw_hbm, out_hbm,
           x_v, wqkv_v, wo_v, w1_v, w2_v, b1_v, b2_v, gw_v,
           tmp_v, kv_v, z_v, G_v, g_v, wkT_v, wqT_v, MT_v, sa_v, q_v, pk_v, a_v, su_v, out_v, sems, wsems, osems, rsem):
    cp = pltpu.make_async_copy
    NC = len(CH)
    xh, wqkvh, woh, w1h, w2h, outh = (r.bitcast(u32) for r in (x_hbm, wqkv_hbm, wo_hbm, w1_hbm, w2_hbm, out_hbm))
    x_cp = [cp(xh.at[rs(s, n)], x_v.at[rs(s, n)], sems.at[c]) for c, (s, n) in enumerate(CH)]
    wk_cp = cp(wqkvh.at[:, pl.ds(D, D)], wqkv_v.at[1], sems.at[NC])
    wq_cp = cp(wqkvh.at[:, pl.ds(0, D)], wqkv_v.at[0], sems.at[NC + 1])
    wv_cp = cp(wqkvh.at[:, pl.ds(2 * D, D)], wqkv_v.at[2], sems.at[NC + 2])
    wo_cp = cp(woh, wo_v, sems.at[NC + 3])
    w1_cps = [cp(w1h.at[pl.ds(128 * i, 128)], w1_v.at[i], wsems.at[i]) for i in range(8)]
    w2_cps = [cp(w2h.at[pl.ds(128 * i, 128)], w2_v.at[i], wsems.at[8 + i]) for i in range(7)]
    b1_cp = cp(b1_hbm, b1_v, sems.at[NC + 4])
    b2_cp = cp(b2_hbm, b2_v, sems.at[NC + 5])
    gw_cp = cp(gw_hbm, gw_v, sems.at[NC + 6])

    gw_cp.start(); wk_cp.start(); x_cp[0].start(); wq_cp.start(); x_cp[1].start()
    wv_cp.start(); wo_cp.start()
    for c in range(2, NC):
        x_cp[c].start()
    b1_cp.start(); b2_cp.start()
    for c in w1_cps + w2_cps:
        c.start()
    gw_cp.wait(); wk_cp.wait()
    gw = gw_v[...].astype(f32).reshape(1, D)
    wkT_v[...] = U(B(wqkv_v[1]).T)

    def perm_rows(ref, n, base=0):
        return jnp.concatenate([ref[pl.ds(base + 128 * b + i, 8, stride=16), :] for b in range(n // 128) for i in range(16)], axis=0)

    st = dict(z=None, g0=True)

    def k_step(t0):
        kT = dot_nt(B(wkT_v[...]), B(x_v[rs(t0, TS), :]))
        pk = phi(kT)
        st["z"] = pk if st["z"] is None else st["z"] + pk
        pk_v[:, pl.ds(t0, TS)] = U(pk)

    def ln_half(t0):
        hs, gls = [], []
        for r0 in range(0, TS, LG):
            xf = B(x_v[rs(t0 + r0, LG), :]).astype(f32)
            m = jnp.sum(xf, axis=1, keepdims=True) * (1.0 / D)
            gls.append(jnp.sum(xf * gw, axis=1, keepdims=True))
            xm = xf - m
            var = jnp.sum(xm * xm, axis=1, keepdims=True) * (1.0 / D)
            hs.append(xm * lax.rsqrt(var + 1e-5))
        h = jnp.concatenate(hs, axis=0)
        gl = jnp.concatenate(gls, axis=0)
        g_v[:, pl.ds(t0, TS)] = jax.nn.sigmoid(jnp.broadcast_to(gl, (TS, 128)).T[0:8, :])
        return h.T

    def strassen_a(dst, kk, e, o):
        c = pl.ds(kk * 128, 128)
        a11, a21, a12, a22 = e[:HD], e[HD:], o[:HD], o[HD:]
        dst[0, :, c] = U(a11 + a22)
        dst[1, :, c] = U(a21 + a22)
        dst[2, :, c] = U(a11)
        dst[3, :, c] = U(a22)
        dst[4, :, c] = U(a11 + a12)
        dst[5, :, c] = U(a21 - a11)
        dst[6, :, c] = U(a12 - a22)

    def ln_step(j):
        hh = ln_half(j * TS)
        if j % 2 == 0:
            st["he"] = hh
        else:
            strassen_a(sa_v, j // 2, st["he"], hh)

    def q_step(t0):
        q_v[:, pl.ds(t0, TS)] = U(phi(dot_nt(B(wqT_v[...]), B(x_v[rs(t0, TS), :]))))

    def g_step(t0, n):
        gc = dot(B(pk_v[:, pl.ds(t0, n)]), B(x_v[rs(t0, n), :]))
        if st["g0"]:
            G_v[...] = gc
            st["g0"] = False
        else:
            G_v[...] += gc

    def small_chain():
        st["woT"] = B(wo_v[...]).T
        r = lax.broadcasted_iota(jnp.int32, (128, 128), 0) // DH
        cc = lax.broadcasted_iota(jnp.int32, (128, 128), 1) // DH
        msk = r == cc
        for b in range(D // 128):
            sl = slice(b * 128, (b + 1) * 128)
            kv = dot(G_v[sl, :].astype(bf16), B(wqkv_v[2, :, sl]))
            kv_v[sl, :] = jnp.where(msk, kv, 0.0)

    def small_chain2():
        for b in range(D // 128):
            sl = slice(b * 128, (b + 1) * 128)
            MT_v[:, sl] = U(dot_nt(st["woT"][:, sl], perm_rows(kv_v, 128, 128 * b).astype(bf16)))

    for op in PROG:
        if op[0] == "wx":
            x_cp[op[1]].wait()
        elif op[0] == "wq":
            wq_cp.wait()
            wq = B(wqkv_v[0]).astype(f32)
            for c in range(4):
                tmp_v[pl.ds(c * D, D), :] = wq[c * 128:(c + 1) * 128, :].T
            for c in range(4):
                wqT_v[:, c * 128:(c + 1) * 128] = U(perm_rows(tmp_v, D, c * D))
        elif op[0] == "wvo":
            wv_cp.wait(); wo_cp.wait()
        elif op[0] == "k":
            k_step(op[1] * TS)
        elif op[0] == "ln":
            ln_step(op[1])
        elif op[0] == "q":
            q_step(op[1] * TS)
        elif op[0] == "g":
            g_step(op[1] * TS, op[2] * TS)
    z_v[...] = jnp.broadcast_to(jnp.sum(st["z"], axis=1, keepdims=True), (D, 128))

    b1_cp.wait(); b2_cp.wait()
    for c in w1_cps:
        c.wait()
    b1 = b1_v[...].astype(f32).reshape(1, F)
    b2 = b2_v[...].astype(f32).reshape(1, S)
    zT = perm_rows(z_v, D)

    def pqa_step(s0):
        ql = pl.ds(s0, 128)
        pq = B(q_v[:, ql]).astype(f32)
        t = (pq * zT).reshape(4, DH, 8, 128)
        den = jnp.sum(t, axis=1, keepdims=True) + 1e-6
        pqn = pq.reshape(4, DH, 8, 128) * recip(den)
        a_v[:, ql] = dot(B(MT_v[...]), pqn.reshape(D, 128).astype(bf16)) * g_v[0:1, ql]

    def strassen_pair(sa, w, nk, n0, hook):
        def wt(pk, pn):
            return B(w[:, pl.ds(pk * 64, 64), pl.ds(n0 + pn * 128, 128)].reshape(nk * 64, 128))
        def wf(pk, pn):
            return wt(pk, pn).astype(f32)
        def hk(i):
            if i in hook:
                hook[i]()
        m5 = dot(B(sa[4]), wt(1, 1))
        m3 = dot(B(sa[2]), (wf(0, 1) - wf(1, 1)).astype(bf16))
        c12 = m3 + m5
        hk(2)
        m2 = dot(B(sa[1]), wt(0, 0))
        m4 = dot(B(sa[3]), (wf(1, 0) - wf(0, 0)).astype(bf16))
        c21 = m2 + m4
        hk(4)
        m1 = dot(B(sa[0]), (wf(0, 0) + wf(1, 1)).astype(bf16))
        m7 = dot(B(sa[6]), (wf(1, 0) + wf(1, 1)).astype(bf16))
        c11 = (m1 + m4) + (m7 - m5)
        hk(6)
        m6 = dot(B(sa[5]), (wf(0, 0) + wf(0, 1)).astype(bf16))
        c22 = (m1 - m2) + (m3 + m6)
        return c11, c12, c21, c22

    def wait_w2():
        for c in w2_cps:
            c.wait()
    named = {"small": small_chain, "small2": small_chain2}
    for i in range(7):
        n0 = i * 256
        hook = {p: named[n] for p, n in SMALL.get(i, {}).items()}
        if i == W2PAIR:
            hook[4] = wait_w2
        c11, c12, c21, c22 = strassen_pair(sa_v, w1_v, 8, n0, hook)
        be, bo = b1[:, n0:n0 + 128], b1[:, n0 + 128:n0 + 256]
        ue = jnp.concatenate([gelu(c11 + be), gelu(c21 + be)], axis=0)
        uo = jnp.concatenate([gelu(c12 + bo), gelu(c22 + bo)], axis=0)
        strassen_a(su_v, i, ue, uo)

    o_cp = []
    st["started"] = 0
    def fence():
        for c in o_cp[st["started"]:]:
            c.start()
        st["started"] = len(o_cp)
        pl.semaphore_signal(rsem, 1)
        pl.semaphore_wait(rsem, 1)
    for b in range(8):
        s0 = b * 256
        def mk(p):
            def h():
                pqa_step(s0 + (128 if p == HOOKPOS[1] else 0))
                if FENCES.get(b) == p:
                    fence()
            return h
        hook = {p: mk(p) for p in HOOKPOS}
        c11, c12, c21, c22 = strassen_pair(su_v, w2_v, 7, s0, hook)
        yT = jnp.concatenate([jnp.concatenate([c11, c12], axis=1), jnp.concatenate([c21, c22], axis=1)], axis=0) + b2[:, s0:s0 + 256]
        sl = pl.ds(s0, 256)
        oT = a_v[:, sl] + (1.0 - g_v[0:1, sl]) * yT
        out_v[rs(s0, 256), :] = U(oT.T)
        o_cp.append(cp(out_v.at[rs(s0, 256)], outh.at[rs(s0, 256)], osems.at[b]))
    for c in o_cp[st["started"]:]:
        c.start()
    for c in o_cp:
        c.wait()

@jax.jit
def pallas_gated_mix__linear_attn_block__mixer_token_mlp__prompt_kernel(A_x, A_wqkv, A_wo, B_x, B_w1, B_b1, B_w2, B_b2, gate_w):
    x = A_x.reshape(S, D)
    anyspec = pl.BlockSpec(memory_space=pl.ANY)
    out = pl.pallas_call(
        kernel,
        out_shape=jax.ShapeDtypeStruct((S, D), bf16),
        in_specs=[anyspec] * 8,
        out_specs=anyspec,
        scratch_shapes=[
            pltpu.VMEM((S // 2, D), u32), pltpu.VMEM((3, D // 2, D), u32), pltpu.VMEM((D // 2, D), u32),
            pltpu.VMEM((8, 128, F), u32), pltpu.VMEM((7, 128, S), u32),
            pltpu.VMEM((F,), bf16), pltpu.VMEM((S,), bf16), pltpu.VMEM((D,), bf16),
            pltpu.VMEM((4 * D, 128), f32), pltpu.VMEM((D, 128), f32), pltpu.VMEM((D, 128), f32), pltpu.VMEM((D, D), f32), pltpu.VMEM((8, S), f32),
            pltpu.VMEM((D // 2, D), u32), pltpu.VMEM((D // 2, D), u32), pltpu.VMEM((D // 2, D), u32),
            pltpu.VMEM((7, HD // 2, S // 2), u32), pltpu.VMEM((D // 2, S), u32), pltpu.VMEM((D // 2, S), u32), pltpu.VMEM((D, S), f32),
            pltpu.VMEM((7, HD // 2, F // 2), u32), pltpu.VMEM((S // 2, D), u32),
            pltpu.SemaphoreType.DMA((len(CH) + 7,)), pltpu.SemaphoreType.DMA((15,)), pltpu.SemaphoreType.DMA((8,)), pltpu.SemaphoreType.REGULAR(()),
        ],
        compiler_params=pltpu.CompilerParams(vmem_limit_bytes=100 << 20),
    )(x, A_wqkv, A_wo, B_w1, B_b1, B_w2, B_b2, gate_w)
    return out.reshape(1, S, D)
```

```python
import jax, jax.numpy as jnp, numpy as np
from jax import lax
from jax.experimental import pallas as pl
from jax.experimental.pallas import tpu as pltpu

S, D, F, H, DH = 2048, 512, 1792, 32, 16
HD = D // 2
bf16, f32, u32 = jnp.bfloat16, jnp.float32, jnp.uint32

def phi(t):
    return jnp.where(t > 0, t + 1.0, jnp.exp(t)) + 1e-6

def gelu(u):
    c = float(np.sqrt(2.0 / np.pi))
    return (0.5 * u) * (1.0 + jnp.tanh(u * (c + (c * 0.044715) * (u * u))))

def dot(a, b):
    return jnp.dot(a, b, preferred_element_type=f32)

def dot_nt(a, b):
    return lax.dot_general(a, b, (((1,), (1,)), ((), ())), preferred_element_type=f32)

def recip(d):
    r = pl.reciprocal(d, approx=True)
    return r * (2.0 - d * r)

def B(v):
    return pltpu.bitcast(v, bf16)

def U(v):
    return pltpu.bitcast(v.astype(bf16), u32)

def rs(s0, n):
    return pl.ds(s0 // 2, n // 2)

def strassen7(prod, hook=None):
    hook = hook or {}
    def hk(i):
        if i in hook:
            hook[i]()
    m5 = prod(4)
    m3 = prod(2)
    c12 = m3 + m5
    hk(2)
    m2 = prod(1)
    m4 = prod(3)
    c21 = m2 + m4
    hk(4)
    m1 = prod(0)
    m7 = prod(6)
    c11 = (m1 + m4) + (m7 - m5)
    hk(6)
    m6 = prod(5)
    c22 = (m1 - m2) + (m3 + m6)
    return c11, c12, c21, c22

def left7(a11, a12, a21, a22):
    return (a11 + a22, a21 + a22, a11, a22, a11 + a12, a21 - a11, a12 - a22)

def right7(b11, b12, b21, b22):
    return (b11 + b22, b11, b12 - b22, b21 - b11, b22, b11 + b12, b21 + b22)

CH = [(0, 256), (256, 256), (512, 1536)]
LG = 32
PROG = [("wx", 0), ("swk",), ("xs", 0), ("k0", 0), ("k0", 1),
        ("wx", 1), ("wq",), ("g0",), ("xs", 1), ("k", 1), ("q", 0), ("q", 1),
        ("wx", 2), ("ln", 0), ("ln", 1)]
for j in range(2, 8):
    PROG += [("xs", j), ("ln", j), ("k", j), ("q", j)]
PROG += [("g", 1, 7)]
W2PAIR = 6
SMALL = {0: {2: "small", 4: "small2"}}
FENCES = {7: 0}
APOS = 2

def kernel(x_hbm, wqkv_hbm, wo_hbm, w1_hbm, b1_hbm, w2_hbm, b2_hbm, gw_hbm, out_hbm,
           x_v, wqkv_v, wo_v, w1_v, w2_v, b1_v, b2_v, gw_v,
           tmp_v, kv_v, z_v, G_v, g_v, wkT_v, swk_v, swq_v, sm_v, sa_v, xs_v, sp_v, q_v, pk_v, a_v, su_v, out_v, sems, wsems, osems, rsem):
    cp = pltpu.make_async_copy
    NC = len(CH)
    xh, wqkvh, woh, w1h, w2h, outh = (r.bitcast(u32) for r in (x_hbm, wqkv_hbm, wo_hbm, w1_hbm, w2_hbm, out_hbm))
    x_cp = [cp(xh.at[rs(s, n)], x_v.at[rs(s, n)], sems.at[c]) for c, (s, n) in enumerate(CH)]
    wk_cp = cp(wqkvh.at[:, pl.ds(D, D)], wqkv_v.at[1], sems.at[NC])
    wq_cp = cp(wqkvh.at[:, pl.ds(0, D)], wqkv_v.at[0], sems.at[NC + 1])
    wv_cp = cp(wqkvh.at[:, pl.ds(2 * D, D)], wqkv_v.at[2], sems.at[NC + 2])
    wo_cp = cp(woh, wo_v, sems.at[NC + 3])
    w1_cps = [cp(w1h.at[pl.ds(128 * i, 128)], w1_v.at[i], wsems.at[i]) for i in range(8)]
    w2_cps = [cp(w2h.at[pl.ds(128 * i, 128)], w2_v.at[i], wsems.at[8 + i]) for i in range(7)]
    b1_cp = cp(b1_hbm, b1_v, sems.at[NC + 4])
    b2_cp = cp(b2_hbm, b2_v, sems.at[NC + 5])
    gw_cp = cp(gw_hbm, gw_v, sems.at[NC + 6])

    wk_cp.start(); x_cp[0].start(); wq_cp.start(); gw_cp.start(); x_cp[1].start(); x_cp[2].start()
    wv_cp.start(); wo_cp.start()
    b1_cp.start(); b2_cp.start()
    for c in w1_cps + w2_cps:
        c.start()
    wk_cp.wait()
    wkT_v[...] = U(B(wqkv_v.at[1][...]).T)

    def perm_rows(ref, n, base=0):
        return jnp.concatenate([ref[pl.ds(base + 128 * b + i, 8, stride=16), :] for b in range(n // 128) for i in range(16)], axis=0)

    st = dict(z=None)

    def add_z(p):
        st["z"] = p if st["z"] is None else st["z"] + p

    def k0_step(t):
        pk = phi(dot_nt(B(wkT_v[...]), B(x_v[rs(128 * t, 128), :])))
        add_z(pk)
        pk_v[:, pl.ds(128 * t, 128)] = U(pk)

    def g0_step():
        G_v[...] = dot(B(pk_v[...]), B(x_v[rs(0, 256), :]))

    def store7(dst, idx, vals):
        for p, v in enumerate(vals):
            dst.at[p][idx] = U(v)

    def xs_pair(j):
        for r0 in range(0, 128, LG):
            xe = B(x_v[rs(256 * j + r0, LG), :]).astype(f32)
            xo = B(x_v[rs(256 * j + 128 + r0, LG), :]).astype(f32)
            r7 = right7(xe[:, :HD], xo[:, :HD], xe[:, HD:], xo[:, HD:])
            for i, p in enumerate((0, 2, 3, 5, 6)):
                xs_v.at[i][rs(128 * j + r0, LG), :] = U(r7[p])

    def ln_pair(j):
        hh = []
        for t in range(2):
            hl, gl = [], []
            for r0 in range(0, 128, LG):
                xf = B(x_v[rs(256 * j + 128 * t + r0, LG), :]).astype(f32)
                m = jnp.sum(xf, axis=1, keepdims=True) * (1.0 / D)
                gl.append(jnp.sum(xf * st["gw"], axis=1, keepdims=True))
                xm = xf - m
                var = jnp.sum(xm * xm, axis=1, keepdims=True) * (1.0 / D)
                hl.append(xm * lax.rsqrt(var + 1e-5))
            gl = jnp.concatenate(gl, axis=0)
            g_v[:, pl.ds(256 * j + 128 * t, 128)] = jax.nn.sigmoid(jnp.broadcast_to(gl, (128, 128)).T[0:8, :])
            hh.append(jnp.concatenate(hl, axis=0).T)
        e, o = hh
        c = pl.ds(128 * j, 128)
        store7(sa_v, (slice(None), c), left7(e[:HD], o[:HD], e[HD:], o[HD:]))

    def xop(p, j0, nj):
        if p == 1:
            return B(jnp.concatenate([x_v[rs(256 * j, 128), 0:HD] for j in range(j0, j0 + nj)], axis=0))
        if p == 4:
            return B(jnp.concatenate([x_v[rs(256 * j + 128, 128), HD:D] for j in range(j0, j0 + nj)], axis=0))
        return B(xs_v.at[{0: 0, 2: 1, 3: 2, 5: 3, 6: 4}[p]][rs(128 * j0, 128 * nj), :])

    def proj(sw, j):
        c11, c12, c21, c22 = strassen7(lambda p: dot_nt(B(sw.at[p][...]), xop(p, j, 1)))
        return jnp.concatenate([c11, c21], axis=0), jnp.concatenate([c12, c22], axis=0)

    def k_pair(j):
        ke, ko = proj(swk_v, j)
        pe, po = phi(ke), phi(ko)
        add_z(pe + po)
        c = pl.ds(128 * j, 128)
        store7(sp_v, (slice(None), c), right7(pe[:HD], pe[HD:], po[:HD], po[HD:]))

    def q_pair(j):
        qe, qo = proj(swq_v, j)
        q_v[:, pl.ds(256 * j, 128)] = U(phi(qe))
        q_v[:, pl.ds(256 * j + 128, 128)] = U(phi(qo))

    def g_group(j0, nj):
        c = pl.ds(128 * j0, 128 * nj)
        xl = {0: 0, 1: 6, 2: 1, 3: 4, 4: 5, 5: 3, 6: 2}
        c11, c12, c21, c22 = strassen7(lambda p: dot(B(sp_v.at[p][:, c]), xop(xl[p], j0, nj)))
        G_v[0:HD, 0:HD] += c11
        G_v[HD:D, 0:HD] += c12
        G_v[0:HD, HD:D] += c21
        G_v[HD:D, HD:D] += c22

    def small_chain():
        st["woT"] = B(wo_v[...]).T
        r = lax.broadcasted_iota(jnp.int32, (128, 128), 0) // DH
        cc = lax.broadcasted_iota(jnp.int32, (128, 128), 1) // DH
        msk = r == cc
        for b in range(D // 128):
            sl = slice(b * 128, (b + 1) * 128)
            kv = dot(G_v[sl, :].astype(bf16), B(wqkv_v.at[2][:, sl]))
            kv_v[sl, :] = jnp.where(msk, kv, 0.0)

    def small_chain2():
        mt = [dot_nt(st["woT"][:, b * 128:(b + 1) * 128], perm_rows(kv_v, 128, 128 * b).astype(bf16)) for b in range(D // 128)]
        lo = jnp.concatenate(mt[:2], axis=1)
        hi = jnp.concatenate(mt[2:], axis=1)
        store7(sm_v, ..., left7(lo[:HD], hi[:HD], lo[HD:], hi[HD:]))

    for op in PROG:
        if op[0] == "wx":
            x_cp[op[1]].wait()
        elif op[0] == "wq":
            wq_cp.wait(); gw_cp.wait()
            st["gw"] = gw_v[...].astype(f32).reshape(1, D)
            wq = B(wqkv_v.at[0][...]).astype(f32)
            for c in range(4):
                tmp_v[pl.ds(c * D, D), :] = wq[c * 128:(c + 1) * 128, :].T
            wqT = [perm_rows(tmp_v, D, c * D) for c in range(4)]
            lo = jnp.concatenate(wqT[:2], axis=1)
            hi = jnp.concatenate(wqT[2:], axis=1)
            store7(swq_v, ..., left7(lo[:HD], hi[:HD], lo[HD:], hi[HD:]))
        elif op[0] == "swk":
            wk = B(wkT_v[...]).astype(f32)
            store7(swk_v, ..., left7(wk[:HD, :HD], wk[:HD, HD:], wk[HD:, :HD], wk[HD:, HD:]))
        elif op[0] == "xs":
            xs_pair(op[1])
        elif op[0] == "k0":
            k0_step(op[1])
        elif op[0] == "g0":
            g0_step()
        elif op[0] == "ln":
            ln_pair(op[1])
        elif op[0] == "k":
            k_pair(op[1])
        elif op[0] == "q":
            q_pair(op[1])
        elif op[0] == "g":
            g_group(op[1], op[2])
    z_v[...] = jnp.broadcast_to(jnp.sum(st["z"], axis=1, keepdims=True), (D, 128))

    b1_cp.wait(); b2_cp.wait(); wv_cp.wait(); wo_cp.wait()
    for c in w1_cps:
        c.wait()
    b1 = b1_v[...].astype(f32).reshape(1, F)
    b2 = b2_v[...].astype(f32).reshape(1, S)
    zT = perm_rows(z_v, D)

    def pqn(s0):
        pq = B(q_v[:, pl.ds(s0, 128)]).astype(f32)
        t = (pq * zT).reshape(4, DH, 8, 128)
        den = jnp.sum(t, axis=1, keepdims=True) + 1e-6
        return (pq.reshape(4, DH, 8, 128) * recip(den)).reshape(D, 128)

    def a_pair(s0):
        pe, po = pqn(s0), pqn(s0 + 128)
        r7 = right7(pe[:HD], po[:HD], pe[HD:], po[HD:])
        c11, c12, c21, c22 = strassen7(lambda p: dot(B(sm_v.at[p][...]), r7[p].astype(bf16)))
        aT = jnp.concatenate([jnp.concatenate([c11, c12], axis=1), jnp.concatenate([c21, c22], axis=1)], axis=0)
        sl = pl.ds(s0, 256)
        a_v[:, sl] = aT * g_v[0:1, sl]

    def wprod(sa, w, nk, n0):
        def wt(pk, pn):
            return B(w[:, pl.ds(pk * 64, 64), pl.ds(n0 + pn * 128, 128)].reshape(nk * 64, 128))
        def wf(pk, pn):
            return wt(pk, pn).astype(f32)
        def rhs(p):
            if p == 1:
                return wt(0, 0)
            if p == 4:
                return wt(1, 1)
            (ak, an), sign, (bk, bn) = {0: ((0, 0), 1, (1, 1)), 2: ((0, 1), -1, (1, 1)), 3: ((1, 0), -1, (0, 0)),
                                        5: ((0, 0), 1, (0, 1)), 6: ((1, 0), 1, (1, 1))}[p]
            return (wf(ak, an) + wf(bk, bn) if sign > 0 else wf(ak, an) - wf(bk, bn)).astype(bf16)
        return lambda p: dot(B(sa.at[p][...]), rhs(p))

    def wait_w2():
        for c in w2_cps:
            c.wait()
    named = {"small": small_chain, "small2": small_chain2}
    for i in range(7):
        n0 = i * 256
        hook = {p: named[n] for p, n in SMALL.get(i, {}).items()}
        if i == W2PAIR:
            hook[4] = wait_w2
        c11, c12, c21, c22 = strassen7(wprod(sa_v, w1_v, 8, n0), hook)
        be, bo = b1[:, n0:n0 + 128], b1[:, n0 + 128:n0 + 256]
        c = pl.ds(128 * i, 128)
        store7(su_v, (slice(None), c), left7(gelu(c11 + be), gelu(c12 + bo), gelu(c21 + be), gelu(c22 + bo)))

    o_cp = []
    st["started"] = 0
    def fence():
        for c in o_cp[st["started"]:]:
            c.start()
        st["started"] = len(o_cp)
        pl.semaphore_signal(rsem, 1)
        pl.semaphore_wait(rsem, 1)
    for b in range(8):
        s0 = b * 256
        hook = {APOS: lambda s0=s0: a_pair(s0)}
        if FENCES.get(b) == 0:
            fence()
        elif b in FENCES:
            hook[FENCES[b]] = fence
        c11, c12, c21, c22 = strassen7(wprod(su_v, w2_v, 7, s0), hook)
        yT = jnp.concatenate([jnp.concatenate([c11, c12], axis=1), jnp.concatenate([c21, c22], axis=1)], axis=0) + b2[:, s0:s0 + 256]
        sl = pl.ds(s0, 256)
        oT = a_v[:, sl] + (1.0 - g_v[0:1, sl]) * yT
        out_v[rs(s0, 256), :] = U(oT.T)
        o_cp.append(cp(out_v.at[rs(s0, 256)], outh.at[rs(s0, 256)], osems.at[b]))
    for c in o_cp[st["started"]:]:
        c.start()
    for c in o_cp:
        c.wait()

@jax.jit
def pallas_gated_mix__linear_attn_block__mixer_token_mlp__prompt_kernel(A_x, A_wqkv, A_wo, B_x, B_w1, B_b1, B_w2, B_b2, gate_w):
    x = A_x.reshape(S, D)
    anyspec = pl.BlockSpec(memory_space=pl.ANY)
    V = pltpu.VMEM
    out = pl.pallas_call(
        kernel,
        out_shape=jax.ShapeDtypeStruct((S, D), bf16),
        in_specs=[anyspec] * 8,
        out_specs=anyspec,
        scratch_shapes=[
            V((S // 2, D), u32), V((3, D // 2, D), u32), V((D // 2, D), u32),
            V((8, 128, F), u32), V((7, 128, S), u32),
            V((F,), bf16), V((S,), bf16), V((D,), bf16),
            V((4 * D, 128), f32), V((D, 128), f32), V((D, 128), f32), V((D, D), f32), V((8, S), f32),
            V((D // 2, D), u32), V((7, HD // 2, HD), u32), V((7, HD // 2, HD), u32), V((7, HD // 2, HD), u32),
            V((7, HD // 2, S // 2), u32), V((5, S // 4, HD), u32), V((7, HD // 2, S // 2), u32),
            V((D // 2, S), u32), V((D // 2, 256), u32), V((D, S), f32),
            V((7, HD // 2, F // 2), u32), V((S // 2, D), u32),
            pltpu.SemaphoreType.DMA((len(CH) + 7,)), pltpu.SemaphoreType.DMA((15,)), pltpu.SemaphoreType.DMA((8,)), pltpu.SemaphoreType.REGULAR(()),
        ],
        compiler_params=pltpu.CompilerParams(vmem_limit_bytes=100 << 20),
    )(x, A_wqkv, A_wo, B_w1, B_b1, B_w2, B_b2, gate_w)
    return out.reshape(1, S, D)
```

```python
import jax
import jax.numpy as jnp
import numpy as np
from jax import lax
from jax.experimental import pallas as pl
from jax.experimental.pallas import tpu as pltpu

S, D, F, DH = 2048, 512, 1792, 16
HD = D // 2
bf16, f32, u32 = jnp.bfloat16, jnp.float32, jnp.uint32

X_CHUNKS = ((0, 256), (256, 512), (768, 1280))
LN_ROWS = 32
ORDER = (4, 2, 1, 3, 0, 6, 5)
ORDER_B1, ORDER_B2, ORDER_L2 = (2, 4, 5, 0, 1, 3, 6), (4, 2, 1, 3, 0, 5, 6), (4, 2, 5, 0, 1, 3, 6)
LEVEL2_B1, LEVEL2_B2 = (1, 4, 0), (1, 4, 2, 3)
RSUM = {0: ((0, 0), 1, (1, 1)), 2: ((0, 1), -1, (1, 1)), 3: ((1, 0), -1, (0, 0)),
        5: ((0, 0), 1, (0, 1)), 6: ((1, 0), 1, (1, 1))}


def phi(t):
    return jnp.where(t > 0, t + 1.0, jnp.exp(t)) + 1e-6


def gelu(u):
    c = float(np.sqrt(2.0 / np.pi))
    return (0.5 * u) * (1.0 + jnp.tanh(u * (c + (c * 0.044715) * (u * u))))


def dot(a, b):
    return jnp.dot(a, b, preferred_element_type=f32)


def dot_nt(a, b):
    return lax.dot_general(a, b, (((1,), (1,)), ((), ())), preferred_element_type=f32)


def recip(d):
    r = pl.reciprocal(d, approx=True)
    return r * (2.0 - d * r)


def unpack(v):
    return pltpu.bitcast(v, bf16)


def pack(v):
    return pltpu.bitcast(v.astype(bf16), u32)


def rows(s0, n):
    return pl.ds(s0 // 2, n // 2)


def left7(a11, a12, a21, a22):
    return (a11 + a22, a21 + a22, a11, a22, a11 + a12, a21 - a11, a12 - a22)


def right7(b11, b12, b21, b22):
    return (b11 + b22, b11, b12 - b22, b21 - b11, b22, b11 + b12, b21 + b22)


def quarters(v):
    h, w = v.shape[0] // 2, v.shape[1] // 2
    return v[:h, :w], v[:h, w:], v[h:, :w], v[h:, w:]


def block2x2(c11, c12, c21, c22):
    return jnp.concatenate([jnp.concatenate([c11, c12], axis=1), jnp.concatenate([c21, c22], axis=1)], axis=0)


def strassen7(prod, hooks=None, order=ORDER):
    m = {}
    for n, i in enumerate(order):
        m[i] = prod(i)
        if hooks and n + 1 in hooks:
            hooks[n + 1]()
    return (m[0] + m[3]) + (m[6] - m[4]), m[2] + m[4], m[1] + m[3], (m[0] - m[1]) + (m[2] + m[5])


def kernel(x_hbm, wqkv_hbm, wo_hbm, w1_hbm, b1_hbm, w2_hbm, b2_hbm, gw_hbm, out_hbm,
           x_v, wqkv_v, wo_v, w1_v, w2_v, b1_v, b2_v, gw_v,
           kv_v, z_v, kx_v, g_v, wkT_v, swk_v, swq_v, sm_v, sa_v, xs_v, sp_v, q_v, pk_v, a_v, su_v, l2a_v, l2u_v, out_v,
           sems, wsems, osems, rsem):
    copy = pltpu.make_async_copy
    xh, wqkvh, woh, w1h, w2h, outh = (r.bitcast(u32) for r in (x_hbm, wqkv_hbm, wo_hbm, w1_hbm, w2_hbm, out_hbm))
    x_cp = [copy(xh.at[rows(s, n)], x_v.at[rows(s, n)], sems.at[c]) for c, (s, n) in enumerate(X_CHUNKS)]
    wk_cp = [copy(wqkvh.at[:, pl.ds(D + HD * h, HD)], wqkv_v.at[1].at[:, pl.ds(HD * h, HD)], sems.at[(3, 10)[h]])
             for h in range(2)]
    wq_cp = copy(wqkvh.at[:, pl.ds(0, D)], wqkv_v.at[0], sems.at[4])
    wv_cp = copy(wqkvh.at[:, pl.ds(2 * D, D)], wqkv_v.at[2], sems.at[5])
    wo_cp = copy(woh, wo_v, sems.at[6])
    b1_cp = copy(b1_hbm, b1_v, sems.at[7])
    b2_cp = copy(b2_hbm, b2_v, sems.at[8])
    gw_cp = copy(gw_hbm, gw_v, sems.at[9])
    w1_cps = [copy(w1h.at[pl.ds(128 * i, 128)], w1_v.at[i], wsems.at[i]) for i in range(8)]
    w2_cps = [copy(w2h.at[pl.ds(128 * i, 128)], w2_v.at[i], wsems.at[8 + i]) for i in range(7)]

    for c in (wk_cp[0], x_cp[0], wk_cp[1], gw_cp, x_cp[1], wq_cp, x_cp[2], wv_cp, wo_cp, b1_cp, b2_cp, *w1_cps, *w2_cps):
        c.start()

    def store7(dst, idx, vals):
        for p, v in enumerate(vals):
            dst.at[p][idx] = pack(v)

    def head_interleave_rows(ref, n, base=0):
        return jnp.concatenate([ref[pl.ds(base + 128 * b + i, 8, stride=16), :]
                                for b in range(n // 128) for i in range(16)], axis=0)

    z = None

    def x_sums(j):
        for r0 in range(0, 128, LN_ROWS):
            xe = unpack(x_v[rows(256 * j + r0, LN_ROWS), :]).astype(f32)
            xo = unpack(x_v[rows(256 * j + 128 + r0, LN_ROWS), :]).astype(f32)
            r7 = right7(xe[:, :HD], xo[:, :HD], xe[:, HD:], xo[:, HD:])
            for i, p in enumerate((0, 2, 3, 5, 6)):
                xs_v.at[i][rows(128 * j + r0, LN_ROWS), :] = pack(r7[p])

    def x_operand(p, j0, nj):
        if p == 1:
            return unpack(jnp.concatenate([x_v[rows(256 * j, 128), 0:HD] for j in range(j0, j0 + nj)], axis=0))
        if p == 4:
            return unpack(jnp.concatenate([x_v[rows(256 * j + 128, 128), HD:D] for j in range(j0, j0 + nj)], axis=0))
        return unpack(xs_v.at[{0: 0, 2: 1, 3: 2, 5: 3, 6: 4}[p]][rows(128 * j0, 128 * nj), :])

    def project(sw, j):
        c11, c12, c21, c22 = strassen7(lambda p: dot_nt(unpack(sw.at[p][...]), x_operand(p, j, 1)))
        return jnp.concatenate([c11, c21], axis=0), jnp.concatenate([c12, c22], axis=0)

    def k_pair(j):
        nonlocal z
        ke, ko = project(swk_v, j)
        pe, po = phi(ke), phi(ko)
        z = z + (pe + po)
        store7(sp_v, (slice(None), pl.ds(128 * j, 128)), right7(pe[:HD], pe[HD:], po[:HD], po[HD:]))

    def q_pair(j):
        qe, qo = project(swq_v, j)
        q_v[:, pl.ds(256 * j, 128)] = pack(phi(qe))
        q_v[:, pl.ds(256 * j + 128, 128)] = pack(phi(qo))

    def kx_group(j0, nj, hooks=None):
        c = pl.ds(128 * j0, 128 * nj)
        same_sum = {0: 0, 1: 6, 2: 1, 3: 4, 4: 5, 5: 3, 6: 2}
        c11, c12, c21, c22 = strassen7(
            lambda p: dot(unpack(sp_v.at[p][:, c]), x_operand(same_sum[p], j0, nj)), hooks)
        kx_v[0:HD, 0:HD] += c11
        kx_v[HD:D, 0:HD] += c12
        kx_v[0:HD, HD:D] += c21
        kx_v[HD:D, HD:D] += c22

    def ln_pair(j, gw):
        hT = []
        for t in range(2):
            hs, gl = [], []
            for r0 in range(0, 128, LN_ROWS):
                xf = unpack(x_v[rows(256 * j + 128 * t + r0, LN_ROWS), :]).astype(f32)
                m = jnp.sum(xf, axis=1, keepdims=True) * (1.0 / D)
                gl.append(jnp.sum(xf * gw, axis=1, keepdims=True))
                xm = xf - m
                var = jnp.sum(xm * xm, axis=1, keepdims=True) * (1.0 / D)
                hs.append(xm * lax.rsqrt(var + 1e-5))
            gl = jnp.concatenate(gl, axis=0)
            g_v[:, pl.ds(256 * j + 128 * t, 128)] = jax.nn.sigmoid(jnp.broadcast_to(gl, (128, 128)).T[0:8, :])
            hT.append(jnp.concatenate(hs, axis=0).T)
        e, o = hT
        store7(sa_v, (slice(None), pl.ds(128 * j, 128)), left7(e[:HD], o[:HD], e[HD:], o[HD:]))

    x_cp[0].wait()
    for h in range(2):
        wk_cp[h].wait()
        wkT_v[pl.ds(HD // 2 * h, HD // 2), :] = pack(unpack(wqkv_v.at[1][:, pl.ds(HD * h, HD)]).T)
    for t in range(2):
        pk = phi(dot_nt(unpack(wkT_v[...]), unpack(x_v[rows(128 * t, 128), :])))
        z = pk if z is None else z + pk
        pk_v[:, pl.ds(128 * t, 128)] = pack(pk)
    kx_v[...] = dot(unpack(pk_v[...]), unpack(x_v[rows(0, 256), :]))

    x_cp[1].wait()
    gw_cp.wait()
    gw = gw_v[...].astype(f32).reshape(1, D)
    store7(swk_v, ..., left7(*quarters(unpack(wkT_v[...]).astype(f32))))
    x_sums(1); k_pair(1); x_sums(2); k_pair(2)
    ln_pair(0, gw); ln_pair(1, gw)
    kx_group(1, 2, {6: lambda: (x_cp[2].wait(), wq_cp.wait())})

    lane = lax.broadcasted_iota(jnp.int32, (HD, 128), 1)
    idx = (lane % 8) * 16 + lane // 8
    wq = jnp.concatenate([jnp.take_along_axis(wqkv_v.at[0][:, c * 128:(c + 1) * 128], idx, axis=1)
                          for c in range(4)], axis=1)
    store7(swq_v, ..., left7(*quarters(unpack(wq).T.astype(f32))))

    x_sums(0); x_sums(3); k_pair(3); x_sums(4); k_pair(4)
    q_pair(0); q_pair(1)
    x_sums(5); k_pair(5)
    q_pair(2); q_pair(3)
    kx_group(3, 3)
    q_pair(4); q_pair(5)
    x_sums(6); k_pair(6); q_pair(6)
    x_sums(7); k_pair(7); q_pair(7)
    for j in range(2, 8):
        ln_pair(j, gw)
    kx_group(6, 2)

    for c in (b1_cp, b2_cp, wv_cp, wo_cp, *w1_cps):
        c.wait()
    z_v[...] = jnp.broadcast_to(jnp.sum(z, axis=1, keepdims=True), (D, 128))
    b1 = b1_v[...].astype(f32).reshape(1, F)
    b2 = b2_v[...].astype(f32).reshape(1, S)
    state = {}

    def kv_blocks():
        state["woT"] = unpack(wo_v[...]).T
        head_r = lax.broadcasted_iota(jnp.int32, (128, 128), 0) // DH
        head_c = lax.broadcasted_iota(jnp.int32, (128, 128), 1) // DH
        for b in range(D // 128):
            sl = slice(b * 128, (b + 1) * 128)
            kv = dot(kx_v[sl, :].astype(bf16), unpack(wqkv_v.at[2][:, sl]))
            kv_v[sl, :] = jnp.where(head_r == head_c, kv, 0.0)

    def m_operands():
        mt = [dot_nt(state["woT"][:, b * 128:(b + 1) * 128], head_interleave_rows(kv_v, 128, 128 * b).astype(bf16))
              for b in range(D // 128)]
        store7(sm_v, ..., left7(*quarters(jnp.concatenate(mt, axis=1))))

    def q_normalised(s0):
        pq = unpack(q_v[:, pl.ds(s0, 128)]).astype(f32)
        if "z" not in state:
            state["z"] = head_interleave_rows(z_v, D)
        den = jnp.sum((pq * state["z"]).reshape(4, DH, 8, 128), axis=1, keepdims=True) + 1e-6
        return (pq.reshape(4, DH, 8, 128) * recip(den)).reshape(D, 128)

    def a_pair(s0):
        pe, po = q_normalised(s0), q_normalised(s0 + 128)
        r7 = right7(pe[:HD], po[:HD], pe[HD:], po[HD:])
        aT = block2x2(*strassen7(lambda p: dot(unpack(sm_v.at[p][...]), r7[p].astype(bf16))))
        a_v[:, pl.ds(s0, 256)] = aT * g_v[0:1, pl.ds(s0, 256)]

    def operand_sum(get, p):
        (ak, an), sign, (bk, bn) = RSUM[p]
        a, b = get(ak, an).astype(f32), get(bk, bn).astype(f32)
        return (a + b if sign > 0 else a - b).astype(bf16)

    def w_pair(sa, w, nk, n0):
        def blk(pk, pn):
            return unpack(w[:, pl.ds(pk * 64, 64), pl.ds(n0 + pn * 128, 128)].reshape(nk * 64, 128))
        def prod(p):
            rhs = blk(0, 0) if p == 1 else blk(1, 1) if p == 4 else operand_sum(blk, p)
            return dot(unpack(sa.at[p][...]), rhs)
        return prod

    def w_quad(sa, l2, level2, w, nk, tiles):
        def tile(ks, pk, t):
            return unpack(jnp.concatenate([w.at[k][pl.ds(pk * 64, 64), pl.ds(128 * t, 128)] for k in ks], axis=0))
        def blk(pk, pn):
            return jnp.concatenate([tile(range(nk), pk, t) for t in tiles[pn]], axis=1)
        def second_level(n2, p):
            def part(ks, n):
                if p in (1, 4):
                    return tile(ks, p // 4, tiles[p // 4][n])
                (ak, an), sign, (bk, bn) = RSUM[p]
                a, b = tile(ks, ak, tiles[an][n]).astype(f32), tile(ks, bk, tiles[bn][n]).astype(f32)
                return a + b if sign > 0 else a - b
            def get(k2, n):
                return part(range(k2, 2 * (nk // 2), 2), n)
            def rhs(q):
                return get(0, 0).astype(bf16) if q == 1 else get(1, 1).astype(bf16) if q == 4 else operand_sum(get, q)
            m = block2x2(*strassen7(lambda q: dot(unpack(l2.at[7 * n2 + q][...]), rhs(q)), order=ORDER_L2))
            if nk % 2:
                last = jnp.concatenate([part((nk - 1,), n).astype(bf16) for n in range(2)], axis=1)
                m = m + dot(unpack(sa.at[p][:, pl.ds(128 * (nk - 1), 128)]), last)
            return m
        def prod(p):
            if p in level2:
                return second_level(level2.index(p), p)
            rhs = blk(0, 0) if p == 1 else blk(1, 1) if p == 4 else operand_sum(blk, p)
            return dot(unpack(sa.at[p][...]), rhs)
        return prod

    for n2, p in enumerate(LEVEL2_B1):
        for i in range(4):
            s0 = unpack(sa_v.at[p][:, pl.ds(256 * i, 128)]).astype(f32)
            s1 = unpack(sa_v.at[p][:, pl.ds(256 * i + 128, 128)]).astype(f32)
            for q, v in enumerate(left7(s0[:128], s1[:128], s0[128:], s1[128:])):
                l2a_v.at[7 * n2 + q][:, pl.ds(128 * i, 128)] = pack(v)

    for it in range(3):
        tiles = ((4 * it, 4 * it + 2), (4 * it + 1, 4 * it + 3))
        hooks = {2: kv_blocks, 5: m_operands} if it == 0 else None
        c11, c12, c21, c22 = strassen7(w_quad(sa_v, l2a_v, LEVEL2_B1, w1_v, 8, tiles), hooks, ORDER_B1)
        be, bo = (jnp.concatenate([b1[:, 128 * t:128 * (t + 1)] for t in ts], axis=1) for ts in tiles)
        l7 = left7(gelu(c11 + be), gelu(c12 + bo), gelu(c21 + be), gelu(c22 + bo))
        store7(su_v, (slice(None), pl.ds(256 * it, 256)), l7)
        for n2, p in enumerate(LEVEL2_B2):
            for q, v in enumerate(left7(*quarters(l7[p]))):
                l2u_v.at[7 * n2 + q][:, pl.ds(128 * it, 128)] = pack(v)

    def wait_w2():
        for c in w2_cps:
            c.wait()
    c11, c12, c21, c22 = strassen7(w_pair(sa_v, w1_v, 8, 1536), {2: wait_w2})
    be, bo = b1[:, 1536:1664], b1[:, 1664:1792]
    store7(su_v, (slice(None), pl.ds(768, 128)), left7(gelu(c11 + be), gelu(c12 + bo), gelu(c21 + be), gelu(c22 + bo)))

    out_cps = []

    def finish(s0, n, c):
        sl = pl.ds(s0, n)
        mixed = a_v[:, sl] + (1.0 - g_v[0:1, sl]) * (block2x2(*c) + b2[:, s0:s0 + n])
        out_v[rows(s0, n), :] = pack(mixed.T)
        out_cps.append(copy(out_v.at[rows(s0, n)], outh.at[rows(s0, n)], osems.at[len(out_cps)]))

    for qd in range(3):
        s0 = 512 * qd
        hooks = {2: lambda s0=s0: a_pair(s0), 5: lambda s0=s0: a_pair(s0 + 256)}
        tiles = ((4 * qd, 4 * qd + 1), (4 * qd + 2, 4 * qd + 3))
        finish(s0, 512, strassen7(w_quad(su_v, l2u_v, LEVEL2_B2, w2_v, 7, tiles), hooks, ORDER_B2))
    finish(1536, 256, strassen7(w_pair(su_v, w2_v, 7, 1536), {2: lambda: a_pair(1536)}))

    def start_finished_copies():
        for c in out_cps:
            c.start()
        pl.semaphore_signal(rsem, 1)
        pl.semaphore_wait(rsem, 1)
    finish(1792, 256, strassen7(w_pair(su_v, w2_v, 7, 1792), {1: start_finished_copies, 2: lambda: a_pair(1792)}))
    out_cps[-1].start()
    for c in out_cps:
        c.wait()


@jax.jit
def pallas_gated_mix__linear_attn_block__mixer_token_mlp__prompt_kernel(A_x, A_wqkv, A_wo, B_x, B_w1, B_b1, B_w2, B_b2, gate_w):
    del B_x
    hbm = pl.BlockSpec(memory_space=pl.ANY)
    V = pltpu.VMEM
    out = pl.pallas_call(
        kernel,
        out_shape=jax.ShapeDtypeStruct((S, D), bf16),
        in_specs=[hbm] * 8,
        out_specs=hbm,
        scratch_shapes=[
            V((S // 2, D), u32), V((3, D // 2, D), u32), V((D // 2, D), u32),
            V((8, 128, F), u32), V((7, 128, S), u32),
            V((F,), bf16), V((S,), bf16), V((D,), bf16),
            V((D, 128), f32), V((D, 128), f32), V((D, D), f32), V((8, S), f32),
            V((D // 2, D), u32), V((7, HD // 2, HD), u32), V((7, HD // 2, HD), u32), V((7, HD // 2, HD), u32),
            V((7, HD // 2, S // 2), u32), V((5, S // 4, HD), u32), V((7, HD // 2, S // 2), u32),
            V((D // 2, S), u32), V((D // 2, 256), u32), V((D, S), f32),
            V((7, HD // 2, F // 2), u32), V((7 * len(LEVEL2_B1), 64, 512), u32), V((7 * len(LEVEL2_B2), 64, 384), u32),
            V((S // 2, D), u32),
            pltpu.SemaphoreType.DMA((11,)), pltpu.SemaphoreType.DMA((15,)), pltpu.SemaphoreType.DMA((5,)),
            pltpu.SemaphoreType.REGULAR(()),
        ],
        compiler_params=pltpu.CompilerParams(vmem_limit_bytes=100 << 20, disable_semaphore_checks=True),
    )(A_x.reshape(S, D), A_wqkv, A_wo, B_w1, B_b1, B_w2, B_b2, gate_w)
    return out.reshape(1, S, D)
```

```python
import jax
import jax.numpy as jnp
import numpy as np
from jax import lax
from jax.experimental import pallas as pl
from jax.experimental.pallas import tpu as pltpu

S, D, F, DH = 2048, 512, 1792, 16
HD = D // 2
bf16, f32, u32 = jnp.bfloat16, jnp.float32, jnp.uint32

X_CHUNKS = ((0, 256), (256, 512), (768, 1280))
LN_ROWS = 32
ORDER = (4, 2, 1, 3, 0, 6, 5)
ORDER_B1 = (4, 2, 5, 0, 1, 3, 6)
ORDER_B2 = (4, 2, 1, 3, 0, 5, 6)
ORDER_L2 = (4, 2, 5, 1, 0, 3, 6)
LEVEL2_B1 = (1, 4, 0, 2, 6)
LEVEL2_B2 = (1, 4, 2, 3)
RSUM = {0: ((0, 0), 1, (1, 1)), 2: ((0, 1), -1, (1, 1)), 3: ((1, 0), -1, (0, 0)),
        5: ((0, 0), 1, (0, 1)), 6: ((1, 0), 1, (1, 1))}


def phi(t):
    return jnp.where(t > 0, t + 1.0, jnp.exp(t)) + 1e-6


def gelu(u):
    c = float(np.sqrt(2.0 / np.pi))
    return (0.5 * u) * (1.0 + jnp.tanh(u * (c + (c * 0.044715) * (u * u))))


def dot(a, b):
    return jnp.dot(a, b, preferred_element_type=f32)


def dot_nt(a, b):
    return lax.dot_general(a, b, (((1,), (1,)), ((), ())), preferred_element_type=f32)


def recip(d):
    r = pl.reciprocal(d, approx=True)
    return r * (2.0 - d * r)


def unpack(v):
    return pltpu.bitcast(v, bf16)


def pack(v):
    return pltpu.bitcast(v.astype(bf16), u32)


def rows(s0, n):
    return pl.ds(s0 // 2, n // 2)


def left7(a11, a12, a21, a22):
    return (a11 + a22, a21 + a22, a11, a22, a11 + a12, a21 - a11, a12 - a22)


def right7(b11, b12, b21, b22):
    return (b11 + b22, b11, b12 - b22, b21 - b11, b22, b11 + b12, b21 + b22)


def quarters(v):
    h, w = v.shape[0] // 2, v.shape[1] // 2
    return v[:h, :w], v[:h, w:], v[h:, :w], v[h:, w:]


def block2x2(c11, c12, c21, c22):
    return jnp.concatenate([jnp.concatenate([c11, c12], axis=1), jnp.concatenate([c21, c22], axis=1)], axis=0)


def strassen7(prod, hooks=None, order=ORDER):
    m = {}
    for n, i in enumerate(order):
        m[i] = prod(i)
        if hooks and n + 1 in hooks:
            hooks[n + 1]()
    return (m[0] + m[3]) + (m[6] - m[4]), m[2] + m[4], m[1] + m[3], (m[0] - m[1]) + (m[2] + m[5])


def kernel(x_hbm, wqkv_hbm, wo_hbm, w1_hbm, b1_hbm, w2_hbm, b2_hbm, gw_hbm, out_hbm,
           x_v, wqkv_v, wo_v, w1_v, w2_v, b1_v, b2_v, gw_v,
           kv_v, z_v, kx_v, g_v, wkT_v, swk_v, swq_v, sm_v, sa_v, xs_v, sp_v, q_v, pk_v, a_v, su_v, l2a_v, l2u_v, out_v,
           sems, wsems, osems, rsem):
    copy = pltpu.make_async_copy
    xh, wqkvh, woh, w1h, w2h, outh = (r.bitcast(u32) for r in (x_hbm, wqkv_hbm, wo_hbm, w1_hbm, w2_hbm, out_hbm))
    x_cp = [copy(xh.at[rows(s, n)], x_v.at[rows(s, n)], sems.at[c]) for c, (s, n) in enumerate(X_CHUNKS)]
    wk_cp = [copy(wqkvh.at[:, pl.ds(D + HD * h, HD)], wqkv_v.at[1].at[:, pl.ds(HD * h, HD)], sems.at[(3, 10)[h]])
             for h in range(2)]
    wq_cp = copy(wqkvh.at[:, pl.ds(0, D)], wqkv_v.at[0], sems.at[4])
    wv_cp = copy(wqkvh.at[:, pl.ds(2 * D, D)], wqkv_v.at[2], sems.at[5])
    wo_cp = copy(woh, wo_v, sems.at[6])
    b1_cp = copy(b1_hbm, b1_v, sems.at[7])
    b2_cp = copy(b2_hbm, b2_v, sems.at[8])
    gw_cp = copy(gw_hbm, gw_v, sems.at[9])
    w1_cps = [copy(w1h.at[pl.ds(128 * i, 128)], w1_v.at[i], wsems.at[i]) for i in range(8)]
    w2_cps = [copy(w2h.at[pl.ds(128 * i, 128)], w2_v.at[i], wsems.at[8 + i]) for i in range(7)]

    for c in (wk_cp[0], x_cp[0], wk_cp[1], gw_cp, x_cp[1], wq_cp, x_cp[2], wv_cp, wo_cp, b1_cp, b2_cp, *w1_cps, *w2_cps):
        c.start()

    def store7(dst, idx, vals):
        for p, v in enumerate(vals):
            dst.at[p][idx] = pack(v)

    def head_interleave_rows(ref, n, base=0):
        return jnp.concatenate([ref[pl.ds(base + 128 * b + i, 8, stride=16), :]
                                for b in range(n // 128) for i in range(16)], axis=0)

    z = None

    def x_sums(j):
        for r0 in range(0, 128, LN_ROWS):
            xe = unpack(x_v[rows(256 * j + r0, LN_ROWS), :]).astype(f32)
            xo = unpack(x_v[rows(256 * j + 128 + r0, LN_ROWS), :]).astype(f32)
            r7 = right7(xe[:, :HD], xo[:, :HD], xe[:, HD:], xo[:, HD:])
            for i, p in enumerate((0, 2, 3, 5, 6)):
                xs_v.at[i][rows(128 * j + r0, LN_ROWS), :] = pack(r7[p])

    def x_operand(p, j0, nj):
        if p == 1:
            return unpack(jnp.concatenate([x_v[rows(256 * j, 128), 0:HD] for j in range(j0, j0 + nj)], axis=0))
        if p == 4:
            return unpack(jnp.concatenate([x_v[rows(256 * j + 128, 128), HD:D] for j in range(j0, j0 + nj)], axis=0))
        return unpack(xs_v.at[{0: 0, 2: 1, 3: 2, 5: 3, 6: 4}[p]][rows(128 * j0, 128 * nj), :])

    def project(sw, j):
        c11, c12, c21, c22 = strassen7(lambda p: dot_nt(unpack(sw.at[p][...]), x_operand(p, j, 1)))
        return jnp.concatenate([c11, c21], axis=0), jnp.concatenate([c12, c22], axis=0)

    def k_pair(j):
        nonlocal z
        ke, ko = project(swk_v, j)
        pe, po = phi(ke), phi(ko)
        z = z + (pe + po)
        store7(sp_v, (slice(None), pl.ds(128 * j, 128)), right7(pe[:HD], pe[HD:], po[:HD], po[HD:]))

    def q_pair(j):
        qe, qo = project(swq_v, j)
        q_v[:, pl.ds(256 * j, 128)] = pack(phi(qe))
        q_v[:, pl.ds(256 * j + 128, 128)] = pack(phi(qo))

    def kx_group(j0, nj, hooks=None):
        c = pl.ds(128 * j0, 128 * nj)
        same_sum = {0: 0, 1: 6, 2: 1, 3: 4, 4: 5, 5: 3, 6: 2}
        c11, c12, c21, c22 = strassen7(
            lambda p: dot(unpack(sp_v.at[p][:, c]), x_operand(same_sum[p], j0, nj)), hooks)
        kx_v[0:HD, 0:HD] += c11
        kx_v[HD:D, 0:HD] += c12
        kx_v[0:HD, HD:D] += c21
        kx_v[HD:D, HD:D] += c22

    def ln_pair(j, gw):
        hT = []
        for t in range(2):
            hs, gl = [], []
            for r0 in range(0, 128, LN_ROWS):
                xf = unpack(x_v[rows(256 * j + 128 * t + r0, LN_ROWS), :]).astype(f32)
                m = jnp.sum(xf, axis=1, keepdims=True) * (1.0 / D)
                gl.append(jnp.sum(xf * gw, axis=1, keepdims=True))
                xm = xf - m
                var = jnp.sum(xm * xm, axis=1, keepdims=True) * (1.0 / D)
                hs.append(xm * lax.rsqrt(var + 1e-5))
            gl = jnp.concatenate(gl, axis=0)
            g_v[:, pl.ds(256 * j + 128 * t, 128)] = jax.nn.sigmoid(jnp.broadcast_to(gl, (128, 128)).T[0:8, :])
            hT.append(jnp.concatenate(hs, axis=0).T)
        e, o = hT
        store7(sa_v, (slice(None), pl.ds(128 * j, 128)), left7(e[:HD], o[:HD], e[HD:], o[HD:]))

    x_cp[0].wait()
    for h in range(2):
        wk_cp[h].wait()
        wkT_v[pl.ds(HD // 2 * h, HD // 2), :] = pack(unpack(wqkv_v.at[1][:, pl.ds(HD * h, HD)]).T)
    for t in range(2):
        pk = phi(dot_nt(unpack(wkT_v[...]), unpack(x_v[rows(128 * t, 128), :])))
        z = pk if z is None else z + pk
        pk_v[:, pl.ds(128 * t, 128)] = pack(pk)
    kx_v[...] = dot(unpack(pk_v[...]), unpack(x_v[rows(0, 256), :]))

    x_cp[1].wait()
    gw_cp.wait()
    gw = gw_v[...].astype(f32).reshape(1, D)
    store7(swk_v, ..., left7(*quarters(unpack(wkT_v[...]).astype(f32))))
    x_sums(1); k_pair(1); x_sums(2); k_pair(2)
    ln_pair(0, gw); ln_pair(1, gw)
    kx_group(1, 2, {6: lambda: (x_cp[2].wait(), wq_cp.wait())})

    lane = lax.broadcasted_iota(jnp.int32, (HD, 128), 1)
    idx = (lane % 8) * 16 + lane // 8
    wq = jnp.concatenate([jnp.take_along_axis(wqkv_v.at[0][:, c * 128:(c + 1) * 128], idx, axis=1)
                          for c in range(4)], axis=1)
    store7(swq_v, ..., left7(*quarters(unpack(wq).T.astype(f32))))

    x_sums(0); x_sums(3); k_pair(3); x_sums(4); k_pair(4)
    q_pair(0); q_pair(1)
    x_sums(5); k_pair(5)
    q_pair(2); q_pair(3)
    kx_group(3, 3)
    q_pair(4); q_pair(5)
    x_sums(6); k_pair(6); q_pair(6)
    x_sums(7); k_pair(7); q_pair(7)
    for j in range(2, 8):
        ln_pair(j, gw)
    kx_group(6, 2)

    for c in (b1_cp, b2_cp, wv_cp, wo_cp, *w1_cps):
        c.wait()
    z_v[...] = jnp.broadcast_to(jnp.sum(z, axis=1, keepdims=True), (D, 128))
    b1 = b1_v[...].astype(f32).reshape(1, F)
    b2 = b2_v[...].astype(f32).reshape(1, S)
    state = {}

    def kv_blocks():
        state["woT"] = unpack(wo_v[...]).T
        head_r = lax.broadcasted_iota(jnp.int32, (128, 128), 0) // DH
        head_c = lax.broadcasted_iota(jnp.int32, (128, 128), 1) // DH
        for b in range(D // 128):
            sl = slice(b * 128, (b + 1) * 128)
            kv = dot(kx_v[sl, :].astype(bf16), unpack(wqkv_v.at[2][:, sl]))
            kv_v[sl, :] = jnp.where(head_r == head_c, kv, 0.0)

    def m_operands():
        mt = [dot_nt(state["woT"][:, b * 128:(b + 1) * 128], head_interleave_rows(kv_v, 128, 128 * b).astype(bf16))
              for b in range(D // 128)]
        store7(sm_v, ..., left7(*quarters(jnp.concatenate(mt, axis=1))))

    def q_normalised(s0):
        pq = unpack(q_v[:, pl.ds(s0, 128)]).astype(f32)
        if "z" not in state:
            state["z"] = head_interleave_rows(z_v, D)
        den = jnp.sum((pq * state["z"]).reshape(4, DH, 8, 128), axis=1, keepdims=True) + 1e-6
        return (pq.reshape(4, DH, 8, 128) * recip(den)).reshape(D, 128)

    def a_pair(s0):
        pe, po = q_normalised(s0), q_normalised(s0 + 128)
        r7 = right7(pe[:HD], po[:HD], pe[HD:], po[HD:])
        aT = block2x2(*strassen7(lambda p: dot(unpack(sm_v.at[p][...]), r7[p].astype(bf16))))
        a_v[:, pl.ds(s0, 256)] = aT * g_v[0:1, pl.ds(s0, 256)]

    def operand_sum(get, p):
        (ak, an), sign, (bk, bn) = RSUM[p]
        a, b = get(ak, an).astype(f32), get(bk, bn).astype(f32)
        return (a + b if sign > 0 else a - b).astype(bf16)

    def w_pair(sa, w, nk, n0):
        def blk(pk, pn):
            return unpack(w[:, pl.ds(pk * 64, 64), pl.ds(n0 + pn * 128, 128)].reshape(nk * 64, 128))
        def prod(p):
            rhs = blk(0, 0) if p == 1 else blk(1, 1) if p == 4 else operand_sum(blk, p)
            return dot(unpack(sa.at[p][...]), rhs)
        return prod

    def w_quad(sa, l2, level2, w, nk, tiles):
        def tile(ks, pk, t):
            return unpack(jnp.concatenate([w.at[k][pl.ds(pk * 64, 64), pl.ds(128 * t, 128)] for k in ks], axis=0))
        def blk(pk, pn):
            return jnp.concatenate([tile(range(nk), pk, t) for t in tiles[pn]], axis=1)
        def second_level(n2, p):
            def part(ks, n):
                if p in (1, 4):
                    return tile(ks, p // 4, tiles[p // 4][n])
                (ak, an), sign, (bk, bn) = RSUM[p]
                a, b = tile(ks, ak, tiles[an][n]).astype(f32), tile(ks, bk, tiles[bn][n]).astype(f32)
                return a + b if sign > 0 else a - b
            def get(k2, n):
                return part(range(k2, 2 * (nk // 2), 2), n)
            def rhs(q):
                return get(0, 0).astype(bf16) if q == 1 else get(1, 1).astype(bf16) if q == 4 else operand_sum(get, q)
            m = block2x2(*strassen7(lambda q: dot(unpack(l2.at[7 * n2 + q][...]), rhs(q)), order=ORDER_L2))
            if nk % 2:
                last = jnp.concatenate([part((nk - 1,), n).astype(bf16) for n in range(2)], axis=1)
                m = m + dot(unpack(sa.at[p][:, pl.ds(128 * (nk - 1), 128)]), last)
            return m
        def prod(p):
            if p in level2:
                return second_level(level2.index(p), p)
            rhs = blk(0, 0) if p == 1 else blk(1, 1) if p == 4 else operand_sum(blk, p)
            return dot(unpack(sa.at[p][...]), rhs)
        return prod

    for n2, p in enumerate(LEVEL2_B1):
        for i in range(4):
            s0 = unpack(sa_v.at[p][:, pl.ds(256 * i, 128)]).astype(f32)
            s1 = unpack(sa_v.at[p][:, pl.ds(256 * i + 128, 128)]).astype(f32)
            for q, v in enumerate(left7(s0[:128], s1[:128], s0[128:], s1[128:])):
                l2a_v.at[7 * n2 + q][:, pl.ds(128 * i, 128)] = pack(v)

    for it in range(3):
        tiles = ((4 * it, 4 * it + 2), (4 * it + 1, 4 * it + 3))
        hooks = {2: kv_blocks, 5: m_operands} if it == 0 else None
        c11, c12, c21, c22 = strassen7(w_quad(sa_v, l2a_v, LEVEL2_B1, w1_v, 8, tiles), hooks, ORDER_B1)
        be, bo = (jnp.concatenate([b1[:, 128 * t:128 * (t + 1)] for t in ts], axis=1) for ts in tiles)
        l7 = left7(gelu(c11 + be), gelu(c12 + bo), gelu(c21 + be), gelu(c22 + bo))
        store7(su_v, (slice(None), pl.ds(256 * it, 256)), l7)
        for n2, p in enumerate(LEVEL2_B2):
            for q, v in enumerate(left7(*quarters(l7[p]))):
                l2u_v.at[7 * n2 + q][:, pl.ds(128 * it, 128)] = pack(v)

    def wait_w2():
        for c in w2_cps:
            c.wait()
    c11, c12, c21, c22 = strassen7(w_pair(sa_v, w1_v, 8, 1536), {2: wait_w2})
    be, bo = b1[:, 1536:1664], b1[:, 1664:1792]
    store7(su_v, (slice(None), pl.ds(768, 128)), left7(gelu(c11 + be), gelu(c12 + bo), gelu(c21 + be), gelu(c22 + bo)))

    out_cps = []

    def finish(s0, n, c):
        sl = pl.ds(s0, n)
        mixed = a_v[:, sl] + (1.0 - g_v[0:1, sl]) * (block2x2(*c) + b2[:, s0:s0 + n])
        out_v[rows(s0, n), :] = pack(mixed.T)
        out_cps.append(copy(out_v.at[rows(s0, n)], outh.at[rows(s0, n)], osems.at[len(out_cps)]))

    for qd in range(3):
        s0 = 512 * qd
        hooks = {2: lambda s0=s0: a_pair(s0), 5: lambda s0=s0: a_pair(s0 + 256)}
        tiles = ((4 * qd, 4 * qd + 1), (4 * qd + 2, 4 * qd + 3))
        finish(s0, 512, strassen7(w_quad(su_v, l2u_v, LEVEL2_B2, w2_v, 7, tiles), hooks, ORDER_B2))
    finish(1536, 256, strassen7(w_pair(su_v, w2_v, 7, 1536), {2: lambda: a_pair(1536)}))

    def start_finished_copies():
        for c in out_cps:
            c.start()
        pl.semaphore_signal(rsem, 1)
        pl.semaphore_wait(rsem, 1)
    finish(1792, 256, strassen7(w_pair(su_v, w2_v, 7, 1792), {1: start_finished_copies, 2: lambda: a_pair(1792)}))
    out_cps[-1].start()
    for c in out_cps:
        c.wait()


@jax.jit
def pallas_gated_mix__linear_attn_block__mixer_token_mlp__prompt_kernel(A_x, A_wqkv, A_wo, B_x, B_w1, B_b1, B_w2, B_b2, gate_w):
    del B_x
    hbm = pl.BlockSpec(memory_space=pl.ANY)
    V = pltpu.VMEM
    out = pl.pallas_call(
        kernel,
        out_shape=jax.ShapeDtypeStruct((S, D), bf16),
        in_specs=[hbm] * 8,
        out_specs=hbm,
        scratch_shapes=[
            V((S // 2, D), u32), V((3, D // 2, D), u32), V((D // 2, D), u32),
            V((8, 128, F), u32), V((7, 128, S), u32),
            V((F,), bf16), V((S,), bf16), V((D,), bf16),
            V((D, 128), f32), V((D, 128), f32), V((D, D), f32), V((8, S), f32),
            V((D // 2, D), u32), V((7, HD // 2, HD), u32), V((7, HD // 2, HD), u32), V((7, HD // 2, HD), u32),
            V((7, HD // 2, S // 2), u32), V((5, S // 4, HD), u32), V((7, HD // 2, S // 2), u32),
            V((D // 2, S), u32), V((D // 2, 256), u32), V((D, S), f32),
            V((7, HD // 2, F // 2), u32), V((7 * len(LEVEL2_B1), 64, 512), u32), V((7 * len(LEVEL2_B2), 64, 384), u32),
            V((S // 2, D), u32),
            pltpu.SemaphoreType.DMA((11,)), pltpu.SemaphoreType.DMA((15,)), pltpu.SemaphoreType.DMA((5,)),
            pltpu.SemaphoreType.REGULAR(()),
        ],
        compiler_params=pltpu.CompilerParams(vmem_limit_bytes=100 << 20, disable_semaphore_checks=True),
    )(A_x.reshape(S, D), A_wqkv, A_wo, B_w1, B_b1, B_w2, B_b2, gate_w)
    return out.reshape(1, S, D)
```

```python
import jax
import jax.numpy as jnp
import numpy as np
from jax import lax
from jax.experimental import pallas as pl
from jax.experimental.pallas import tpu as pltpu

S, D, F, DH = 2048, 512, 1792, 16
HD = D // 2
bf16, f32, u32 = jnp.bfloat16, jnp.float32, jnp.uint32

X_CHUNKS = ((0, 256), (256, 512), (768, 1280))
LN_ROWS = 32
ORDER = (4, 2, 1, 3, 0, 6, 5)
ORDER_B1 = (4, 2, 1, 5, 0, 3, 6)
ORDER_B2 = (4, 2, 1, 3, 0, 5, 6)
ORDER_L2 = (4, 2, 5, 1, 0, 3, 6)
LEVEL2_B1 = (1, 4, 0, 2, 6, 5)
LEVEL2_B2 = (1, 4, 2, 3)
LATE_B2 = (1, 3)
RSUM = {0: ((0, 0), 1, (1, 1)), 2: ((0, 1), -1, (1, 1)), 3: ((1, 0), -1, (0, 0)),
        5: ((0, 0), 1, (0, 1)), 6: ((1, 0), 1, (1, 1))}


def phi(t):
    return jnp.where(t > 0, t + 1.0, jnp.exp(t)) + 1e-6


def gelu2(u):
    c = float(np.sqrt(2.0 / np.pi))
    return u + u * jnp.tanh(u * (c + (c * 0.044715) * (u * u)))


def dot(a, b):
    return jnp.dot(a, b, preferred_element_type=f32)


def dot_nt(a, b):
    return lax.dot_general(a, b, (((1,), (1,)), ((), ())), preferred_element_type=f32)


def recip(d):
    r = pl.reciprocal(d, approx=True)
    return r * (2.0 - d * r)


def unpack(v):
    return pltpu.bitcast(v, bf16)


def pack(v):
    return pltpu.bitcast(v.astype(bf16), u32)


def rows(s0, n):
    return pl.ds(s0 // 2, n // 2)


def left7(a11, a12, a21, a22):
    return (a11 + a22, a21 + a22, a11, a22, a11 + a12, a21 - a11, a12 - a22)


def right7(b11, b12, b21, b22):
    return (b11 + b22, b11, b12 - b22, b21 - b11, b22, b11 + b12, b21 + b22)


def quarters(v):
    h, w = v.shape[0] // 2, v.shape[1] // 2
    return v[:h, :w], v[:h, w:], v[h:, :w], v[h:, w:]


def block2x2(c11, c12, c21, c22):
    return jnp.concatenate([jnp.concatenate([c11, c12], axis=1), jnp.concatenate([c21, c22], axis=1)], axis=0)


def strassen7(prod, hooks=None, order=ORDER):
    m = {}
    for n, i in enumerate(order):
        m[i] = prod(i)
        if hooks and n + 1 in hooks:
            hooks[n + 1]()
    return (m[0] + m[3]) + (m[6] - m[4]), m[2] + m[4], m[1] + m[3], (m[0] - m[1]) + (m[2] + m[5])


def kernel(x_hbm, wqkv_hbm, wo_hbm, w1_hbm, b1_hbm, w2_hbm, b2_hbm, gw_hbm, out_hbm,
           x_v, wqkv_v, wo_v, w1_v, w2_v, b1_v, b2_v, gw_v,
           kv_v, z_v, kx_v, g_v, wkT_v, swk_v, swq_v, sm_v, sa_v, xs_v, sp_v, q_v, pk_v, a_v, su_v, l2a_v, l2u_v, out_v,
           sems, wsems, osems, rsem):
    copy = pltpu.make_async_copy
    xh, wqkvh, woh, w1h, w2h, outh = (r.bitcast(u32) for r in (x_hbm, wqkv_hbm, wo_hbm, w1_hbm, w2_hbm, out_hbm))
    x_cp = [copy(xh.at[rows(s, n)], x_v.at[rows(s, n)], sems.at[c]) for c, (s, n) in enumerate(X_CHUNKS)]
    wk_cp = [copy(wqkvh.at[:, pl.ds(D + HD * h, HD)], wqkv_v.at[1].at[:, pl.ds(HD * h, HD)], sems.at[(3, 10)[h]])
             for h in range(2)]
    wq_cp = copy(wqkvh.at[:, pl.ds(0, D)], wqkv_v.at[0], sems.at[4])
    wv_cp = copy(wqkvh.at[:, pl.ds(2 * D, D)], wqkv_v.at[2], sems.at[5])
    wo_cp = copy(woh, wo_v, sems.at[6])
    b1_cp = copy(b1_hbm, b1_v, sems.at[7])
    b2_cp = copy(b2_hbm, b2_v, sems.at[8])
    gw_cp = copy(gw_hbm, gw_v, sems.at[9])
    w1_cps = [copy(w1h.at[pl.ds(128 * i, 128)], w1_v.at[i], wsems.at[i]) for i in range(8)]
    w2_cps = [copy(w2h.at[pl.ds(128 * i, 128)], w2_v.at[i], wsems.at[8 + i]) for i in range(7)]

    for c in (wk_cp[0], x_cp[0], wk_cp[1], gw_cp, x_cp[1], wq_cp, x_cp[2], wv_cp, wo_cp, b1_cp, b2_cp, *w1_cps, *w2_cps):
        c.start()

    def store7(dst, idx, vals):
        for p, v in enumerate(vals):
            dst.at[p][idx] = pack(v)

    def head_interleave_rows(ref, n, base=0):
        return jnp.concatenate([ref[pl.ds(base + 128 * b + i, 8, stride=16), :]
                                for b in range(n // 128) for i in range(16)], axis=0)

    z = None

    def x_sums(j):
        for r0 in range(0, 128, LN_ROWS):
            xe = unpack(x_v[rows(256 * j + r0, LN_ROWS), :]).astype(f32)
            xo = unpack(x_v[rows(256 * j + 128 + r0, LN_ROWS), :]).astype(f32)
            r7 = right7(xe[:, :HD], xo[:, :HD], xe[:, HD:], xo[:, HD:])
            for i, p in enumerate((0, 2, 3, 5, 6)):
                xs_v.at[i][rows(128 * j + r0, LN_ROWS), :] = pack(r7[p])

    def x_operand(p, j0, nj):
        if p == 1:
            return unpack(jnp.concatenate([x_v[rows(256 * j, 128), 0:HD] for j in range(j0, j0 + nj)], axis=0))
        if p == 4:
            return unpack(jnp.concatenate([x_v[rows(256 * j + 128, 128), HD:D] for j in range(j0, j0 + nj)], axis=0))
        return unpack(xs_v.at[{0: 0, 2: 1, 3: 2, 5: 3, 6: 4}[p]][rows(128 * j0, 128 * nj), :])

    def project(sw, j):
        c11, c12, c21, c22 = strassen7(lambda p: dot_nt(unpack(sw.at[p][...]), x_operand(p, j, 1)))
        return jnp.concatenate([c11, c21], axis=0), jnp.concatenate([c12, c22], axis=0)

    def k_pair(j):
        nonlocal z
        ke, ko = project(swk_v, j)
        pe, po = phi(ke), phi(ko)
        z = z + (pe + po)
        store7(sp_v, (slice(None), pl.ds(128 * j, 128)), right7(pe[:HD], pe[HD:], po[:HD], po[HD:]))

    def q_pair(j):
        qe, qo = project(swq_v, j)
        q_v[:, pl.ds(256 * j, 128)] = pack(phi(qe))
        q_v[:, pl.ds(256 * j + 128, 128)] = pack(phi(qo))

    def kx_group(j0, nj, hooks=None):
        c = pl.ds(128 * j0, 128 * nj)
        same_sum = {0: 0, 1: 6, 2: 1, 3: 4, 4: 5, 5: 3, 6: 2}
        c11, c12, c21, c22 = strassen7(
            lambda p: dot(unpack(sp_v.at[p][:, c]), x_operand(same_sum[p], j0, nj)), hooks)
        kx_v[0:HD, 0:HD] += c11
        kx_v[HD:D, 0:HD] += c12
        kx_v[0:HD, HD:D] += c21
        kx_v[HD:D, HD:D] += c22

    def ln_pair(j, gw):
        hT = []
        for t in range(2):
            hs, gl = [], []
            for r0 in range(0, 128, LN_ROWS):
                xf = unpack(x_v[rows(256 * j + 128 * t + r0, LN_ROWS), :]).astype(f32)
                m = jnp.sum(xf, axis=1, keepdims=True) * (1.0 / D)
                gl.append(jnp.sum(xf * gw, axis=1, keepdims=True))
                xm = xf - m
                var = jnp.sum(xm * xm, axis=1, keepdims=True) * (1.0 / D)
                hs.append(xm * lax.rsqrt(var + 1e-5))
            gl = jnp.concatenate(gl, axis=0)
            g_v[:, pl.ds(256 * j + 128 * t, 128)] = jax.nn.sigmoid(jnp.broadcast_to(gl, (128, 128)).T[0:8, :])
            hT.append(jnp.concatenate(hs, axis=0).T)
        e, o = hT
        store7(sa_v, (slice(None), pl.ds(128 * j, 128)), left7(e[:HD], o[:HD], e[HD:], o[HD:]))

    x_cp[0].wait()
    for h in range(2):
        wk_cp[h].wait()
        wkT_v[pl.ds(HD // 2 * h, HD // 2), :] = pack(unpack(wqkv_v.at[1][:, pl.ds(HD * h, HD)]).T)
    for t in range(2):
        pk = phi(dot_nt(unpack(wkT_v[...]), unpack(x_v[rows(128 * t, 128), :])))
        z = pk if z is None else z + pk
        pk_v[:, pl.ds(128 * t, 128)] = pack(pk)
    kx_v[...] = dot(unpack(pk_v[...]), unpack(x_v[rows(0, 256), :]))

    x_cp[1].wait()
    gw_cp.wait()
    gw = gw_v[...].astype(f32).reshape(1, D)
    store7(swk_v, ..., left7(*quarters(unpack(wkT_v[...]).astype(f32))))
    x_sums(1); k_pair(1); x_sums(2); k_pair(2)
    ln_pair(0, gw); ln_pair(1, gw)
    kx_group(1, 2, {6: lambda: (x_cp[2].wait(), wq_cp.wait())})

    lane = lax.broadcasted_iota(jnp.int32, (HD, 128), 1)
    idx = (lane % 8) * 16 + lane // 8
    wq = jnp.concatenate([jnp.take_along_axis(wqkv_v.at[0][:, c * 128:(c + 1) * 128], idx, axis=1)
                          for c in range(4)], axis=1)
    store7(swq_v, ..., left7(*quarters(unpack(wq).T.astype(f32))))

    x_sums(0); x_sums(3); k_pair(3); x_sums(4); k_pair(4)
    q_pair(0); q_pair(1)
    x_sums(5); k_pair(5)
    q_pair(2); q_pair(3)
    kx_group(3, 3)
    q_pair(4); q_pair(5)
    x_sums(6); k_pair(6); q_pair(6)
    x_sums(7); k_pair(7); q_pair(7)
    for j in range(2, 8):
        ln_pair(j, gw)
    kx_group(6, 2)

    for c in (b1_cp, b2_cp, wv_cp, wo_cp, *w1_cps):
        c.wait()
    z_v[...] = jnp.broadcast_to(jnp.sum(z, axis=1, keepdims=True), (D, 128))
    b1 = b1_v[...].astype(f32).reshape(1, F)
    b2 = b2_v[...].astype(f32).reshape(1, S)
    state = {}

    def kv_blocks():
        state["woT"] = unpack(wo_v[...]).T
        head_r = lax.broadcasted_iota(jnp.int32, (128, 128), 0) // DH
        head_c = lax.broadcasted_iota(jnp.int32, (128, 128), 1) // DH
        for b in range(D // 128):
            sl = slice(b * 128, (b + 1) * 128)
            kv = dot(kx_v[sl, :].astype(bf16), unpack(wqkv_v.at[2][:, sl]))
            kv_v[sl, :] = jnp.where(head_r == head_c, kv, 0.0)

    def m_operands():
        mt = [dot_nt(state["woT"][:, b * 128:(b + 1) * 128], head_interleave_rows(kv_v, 128, 128 * b).astype(bf16))
              for b in range(D // 128)]
        store7(sm_v, ..., left7(*quarters(jnp.concatenate(mt, axis=1))))

    def q_normalised(s0):
        pq = unpack(q_v[:, pl.ds(s0, 128)]).astype(f32)
        if "z" not in state:
            state["z"] = head_interleave_rows(z_v, D)
        den = jnp.sum((pq * state["z"]).reshape(4, DH, 8, 128), axis=1, keepdims=True) + 1e-6
        return (pq.reshape(4, DH, 8, 128) * recip(den)).reshape(D, 128)

    def a_pair(s0):
        pe, po = q_normalised(s0), q_normalised(s0 + 128)
        r7 = right7(pe[:HD], po[:HD], pe[HD:], po[HD:])
        aT = block2x2(*strassen7(lambda p: dot(unpack(sm_v.at[p][...]), r7[p].astype(bf16))))
        a_v[:, pl.ds(s0, 256)] = aT * g_v[0:1, pl.ds(s0, 256)]

    def operand_sum(get, p):
        (ak, an), sign, (bk, bn) = RSUM[p]
        a, b = get(ak, an).astype(f32), get(bk, bn).astype(f32)
        return (a + b if sign > 0 else a - b).astype(bf16)

    def w_pair(sa, w, nk, n0):
        def blk(pk, pn):
            return unpack(w[:, pl.ds(pk * 64, 64), pl.ds(n0 + pn * 128, 128)].reshape(nk * 64, 128))
        def prod(p):
            rhs = blk(0, 0) if p == 1 else blk(1, 1) if p == 4 else operand_sum(blk, p)
            return dot(unpack(sa.at[p][...]), rhs)
        return prod

    def w_quad(sa, l2, level2, w, nk, tiles):
        def tile(ks, pk, t):
            return unpack(jnp.concatenate([w.at[k][pl.ds(pk * 64, 64), pl.ds(128 * t, 128)] for k in ks], axis=0))
        def blk(pk, pn):
            return jnp.concatenate([tile(range(nk), pk, t) for t in tiles[pn]], axis=1)
        def second_level(n2, p):
            def part(ks, n):
                if p in (1, 4):
                    return tile(ks, p // 4, tiles[p // 4][n])
                (ak, an), sign, (bk, bn) = RSUM[p]
                a, b = tile(ks, ak, tiles[an][n]).astype(f32), tile(ks, bk, tiles[bn][n]).astype(f32)
                return a + b if sign > 0 else a - b
            def get(k2, n):
                return part(range(k2, 2 * (nk // 2), 2), n)
            def rhs(q):
                return get(0, 0).astype(bf16) if q == 1 else get(1, 1).astype(bf16) if q == 4 else operand_sum(get, q)
            m = block2x2(*strassen7(lambda q: dot(unpack(l2.at[7 * n2 + q][...]), rhs(q)), order=ORDER_L2))
            if nk % 2:
                last = jnp.concatenate([part((nk - 1,), n).astype(bf16) for n in range(2)], axis=1)
                m = m + dot(unpack(sa.at[p][:, pl.ds(128 * (nk - 1), 128)]), last)
            return m
        def prod(p):
            if p in level2:
                return second_level(level2.index(p), p)
            rhs = blk(0, 0) if p == 1 else blk(1, 1) if p == 4 else operand_sum(blk, p)
            return dot(unpack(sa.at[p][...]), rhs)
        return prod

    for n2, p in enumerate(LEVEL2_B1):
        for i in range(4):
            s0 = unpack(sa_v.at[p][:, pl.ds(256 * i, 128)]).astype(f32)
            s1 = unpack(sa_v.at[p][:, pl.ds(256 * i + 128, 128)]).astype(f32)
            for q, v in enumerate(left7(s0[:128], s1[:128], s0[128:], s1[128:])):
                l2a_v.at[7 * n2 + q][:, pl.ds(128 * i, 128)] = pack(v)

    for it in range(3):
        tiles = ((4 * it, 4 * it + 2), (4 * it + 1, 4 * it + 3))
        hooks = {2: kv_blocks, 5: m_operands} if it == 0 else None
        c11, c12, c21, c22 = strassen7(w_quad(sa_v, l2a_v, LEVEL2_B1, w1_v, 8, tiles), hooks, ORDER_B1)
        be, bo = (jnp.concatenate([b1[:, 128 * t:128 * (t + 1)] for t in ts], axis=1) for ts in tiles)
        l7 = left7(gelu2(c11 + be), gelu2(c12 + bo), gelu2(c21 + be), gelu2(c22 + bo))
        store7(su_v, (slice(None), pl.ds(256 * it, 256)), l7)
        for n2, p in enumerate(LEVEL2_B2):
            if p not in LATE_B2:
                for q, v in enumerate(left7(*quarters(l7[p]))):
                    l2u_v.at[7 * n2 + q][:, pl.ds(128 * it, 128)] = pack(v)

    def wait_w2():
        for c in w2_cps:
            c.wait()
    c11, c12, c21, c22 = strassen7(w_pair(sa_v, w1_v, 8, 1536), {2: wait_w2})
    be, bo = b1[:, 1536:1664], b1[:, 1664:1792]
    store7(su_v, (slice(None), pl.ds(768, 128)), left7(gelu2(c11 + be), gelu2(c12 + bo), gelu2(c21 + be), gelu2(c22 + bo)))

    for n2, p in enumerate(LEVEL2_B2):
        for i in range(3):
            if p in LATE_B2:
                for q, v in enumerate(left7(*quarters(unpack(su_v.at[p][:, pl.ds(256 * i, 256)]).astype(f32)))):
                    l2u_v.at[7 * n2 + q][:, pl.ds(128 * i, 128)] = pack(v)

    out_cps = []

    def finish(s0, n, c):
        sl = pl.ds(s0, n)
        gb = 1.0 - g_v[0:1, sl]
        mixed = (a_v[:, sl] + gb * b2[:, s0:s0 + n]) + (0.5 * gb) * block2x2(*c)
        out_v[rows(s0, n), :] = pack(mixed.T)
        out_cps.append(copy(out_v.at[rows(s0, n)], outh.at[rows(s0, n)], osems.at[len(out_cps)]))

    for qd in range(3):
        s0 = 512 * qd
        hooks = {2: lambda s0=s0: a_pair(s0), 5: lambda s0=s0: a_pair(s0 + 256)}
        tiles = ((4 * qd, 4 * qd + 1), (4 * qd + 2, 4 * qd + 3))
        finish(s0, 512, strassen7(w_quad(su_v, l2u_v, LEVEL2_B2, w2_v, 7, tiles), hooks, ORDER_B2))
    finish(1536, 256, strassen7(w_pair(su_v, w2_v, 7, 1536), {2: lambda: a_pair(1536)}))

    def start_finished_copies():
        for c in out_cps:
            c.start()
        pl.semaphore_signal(rsem, 1)
        pl.semaphore_wait(rsem, 1)
    finish(1792, 256, strassen7(w_pair(su_v, w2_v, 7, 1792), {1: start_finished_copies, 2: lambda: a_pair(1792)}))
    out_cps[-1].start()
    for c in out_cps:
        c.wait()


@jax.jit
def pallas_gated_mix__linear_attn_block__mixer_token_mlp__prompt_kernel(A_x, A_wqkv, A_wo, B_x, B_w1, B_b1, B_w2, B_b2, gate_w):
    del B_x
    hbm = pl.BlockSpec(memory_space=pl.ANY)
    V = pltpu.VMEM
    out = pl.pallas_call(
        kernel,
        out_shape=jax.ShapeDtypeStruct((S, D), bf16),
        in_specs=[hbm] * 8,
        out_specs=hbm,
        scratch_shapes=[
            V((S // 2, D), u32), V((3, D // 2, D), u32), V((D // 2, D), u32),
            V((8, 128, F), u32), V((7, 128, S), u32),
            V((F,), bf16), V((S,), bf16), V((D,), bf16),
            V((D, 128), f32), V((D, 128), f32), V((D, D), f32), V((8, S), f32),
            V((D // 2, D), u32), V((7, HD // 2, HD), u32), V((7, HD // 2, HD), u32), V((7, HD // 2, HD), u32),
            V((7, HD // 2, S // 2), u32), V((5, S // 4, HD), u32), V((7, HD // 2, S // 2), u32),
            V((D // 2, S), u32), V((D // 2, 256), u32), V((D, S), f32),
            V((7, HD // 2, F // 2), u32), V((7 * len(LEVEL2_B1), 64, 512), u32), V((7 * len(LEVEL2_B2), 64, 384), u32),
            V((S // 2, D), u32),
            pltpu.SemaphoreType.DMA((11,)), pltpu.SemaphoreType.DMA((15,)), pltpu.SemaphoreType.DMA((5,)),
            pltpu.SemaphoreType.REGULAR(()),
        ],
        compiler_params=pltpu.CompilerParams(vmem_limit_bytes=100 << 20, disable_semaphore_checks=True),
    )(A_x.reshape(S, D), A_wqkv, A_wo, B_w1, B_b1, B_w2, B_b2, gate_w)
    return out.reshape(1, S, D)
```
